```python
import jax
import jax.numpy as jnp

def _softmax(x, axis=-1):
    return jax.nn.softmax(x, axis=axis)

def _gelu(x):
    return jax.nn.gelu(x, approximate=True)

def _silu(x):
    return jax.nn.silu(x)

def _sigmoid(x):
    return jax.nn.sigmoid(x)

def _layernorm(x, axis=-1, eps=1e-05):
    m = jnp.mean(x, axis=axis, keepdims=True)
    v = jnp.var(x, axis=axis, keepdims=True)
    return (x - m) / jnp.sqrt(v + eps)

def _scatter_add(tgt, idx, src, axis=0):
    return tgt.at[idx].add(src)

def _segment_sum(src, seg, n):
    return jax.ops.segment_sum(src, seg, n)

class _Rng:

    def __init__(self, key):
        self._k = key

    def _next(self):
        self._k, sub = jax.random.split(self._k)
        return sub

    def normal(self, shape):
        return jax.random.normal(self._next(), shape, dtype=jnp.bfloat16)

    def randint(self, lo, hi, shape):
        return jax.random.randint(self._next(), shape, lo, hi, dtype=jnp.int32)

    def uniform(self, shape, lo=0.0, hi=1.0):
        return jax.random.uniform(self._next(), shape, jnp.bfloat16, lo, hi)

    def permutation(self, n):
        return jax.random.permutation(self._next(), n)
kernel_name = 'gated_mix__memory_aug_recurrent_mem_tr__sliding_local_dilated__prompt'

def setup_inputs():
    _rng = _Rng(jax.random.key(int.from_bytes(__import__("os").urandom(4), "little")))
    _w = lambda a: (lambda t: t.astype(jnp.bfloat16) if jnp.issubdtype(t.dtype, jnp.floating) else t)(jnp.asarray(a))

    def _A_setup():
        B, S, Dm = (1, 2048, 640)
        H, Dh = (32, 192)
        M, seg = (8, 32)
        seg = min(seg, S)
        S = S // seg * seg
        return {'x': _w((lambda *s: _rng.normal(s) * 0.05)(B, S, Dm)), 'mem0': _w((lambda *s: _rng.normal(s) * 0.05)(B, M, Dm)), 'Wq': _w((lambda *s: _rng.normal(s) * 0.05)(Dm, H, Dh) * Dm ** (-0.5)), 'Wk': _w((lambda *s: _rng.normal(s) * 0.05)(Dm, H, Dh) * Dm ** (-0.5)), 'Wv': _w((lambda *s: _rng.normal(s) * 0.05)(Dm, H, Dh) * Dm ** (-0.5)), 'Wo': _w((lambda *s: _rng.normal(s) * 0.05)(H, Dh, Dm) * (H * Dh) ** (-0.5)), 'seg_len': seg}
    _A_in = _A_setup()

    def _B_setup():
        B, S, D = (1, 2048, 640)
        return {'x': _w((lambda *s: _rng.normal(s) * 0.05)(B, S, D)), 'wqkv': _w((lambda *s: _rng.normal(s) * 0.05)(D, 3 * D)), 'wo': _w((lambda *s: _rng.normal(s) * 0.05)(D, D))}
    _B_in = _B_setup()
    return {'A_x': _A_in['x'], 'A_mem0': _A_in['mem0'], 'A_Wq': _A_in['Wq'], 'A_Wk': _A_in['Wk'], 'A_Wv': _A_in['Wv'], 'A_Wo': _A_in['Wo'], 'A_seg_len': _A_in['seg_len'], 'B_x': _B_in['x'], 'B_wqkv': _B_in['wqkv'], 'B_wo': _B_in['wo'], 'gate_w': _w((lambda *s: _rng.normal(s) * 0.05)(640))}

def reference(A_x, A_mem0, A_Wq, A_Wk, A_Wv, A_Wo, A_seg_len, B_x, B_wqkv, B_wo, gate_w):

    def _A_ref(x, mem0, Wq, Wk, Wv, Wo, seg_len):
        B, S, Dm = x.shape
        H, Dh = (Wq.shape[1], Wq.shape[2])
        M = mem0.shape[1]
        scale = Dh ** (-0.5)
        n_seg = S // seg_len
        L = M + seg_len
        idx = jnp.arange(L)
        mask = (idx[:, None] < M) | (idx[:, None] >= idx[None, :])
        mem = mem0
        outs = []
        for s in range(n_seg):
            xs = x[:, s * seg_len:(s + 1) * seg_len, :].copy()
            h = jnp.concatenate([mem, xs], axis=1)
            q = jnp.einsum('btd,dhe->bhte', h, Wq)
            k = jnp.einsum('btd,dhe->bhte', h, Wk)
            v = jnp.einsum('btd,dhe->bhte', h, Wv)
            scores = jnp.einsum('bhqe,bhke->bhqk', q, k) * scale
            scores = jnp.where(mask[None, None], scores, -1000000000.0)
            p = _softmax(scores, axis=-1)
            o = jnp.einsum('bhqk,bhke->bhqe', p, v)
            o = jnp.einsum('bhte,hed->btd', o, Wo)
            mem = o[:, :M, :].copy()
            outs.append(o[:, M:, :])
        return jnp.concatenate(outs, axis=1)

    def _B_ref(x, wqkv, wo):
        B, S, D = x.shape
        H = 32
        Dh = D // H
        W, dil = (8, 2)
        qkv = (lambda x, *d: x.transpose(*d))((x @ wqkv).reshape(B, S, 3, H, Dh), 2, 0, 3, 1, 4)
        q, k, v = (qkv[0], qkv[1], qkv[2])
        scale = Dh ** (-0.5)
        pos = jnp.arange(S)
        off = jnp.arange(W) * dil
        idx = pos[:, None] - off[None, :]
        mask = idx >= 0
        idx_c = jnp.where(mask, idx, 0).reshape(-1)
        kg = k[:, :, idx_c, :].reshape(B, H, S, W, Dh)
        vg = v[:, :, idx_c, :].reshape(B, H, S, W, Dh)
        logits = jnp.einsum('bhsd,bhswd->bhsw', q, kg) * scale
        logits = jnp.where(mask[None, None, :, :], logits, -1000000000.0)
        attn = _softmax(logits, axis=-1)
        o = jnp.einsum('bhsw,bhswd->bhsd', attn, vg)
        return (lambda x, *d: x.transpose(*d))(o, 0, 2, 1, 3).reshape(B, S, D) @ wo
    x = A_x
    g = _sigmoid((x * gate_w).sum(-1, keepdims=True))
    a = _A_ref(x, A_mem0, A_Wq, A_Wk, A_Wv, A_Wo, A_seg_len)
    b = _B_ref(x, B_wqkv, B_wo)
    return g * a + (1 - g) * b
```

```python
import functools

import jax
import jax.numpy as jnp
import jax.experimental.pallas as pl
import jax.experimental.pallas.tpu as pltpu

F32 = jnp.float32
BF16 = jnp.bfloat16
NEG = -1000000000.0
LANES = 128

B_HEADS, B_WIN, B_DIL = 32, 8, 2
B_HALO = 16
B_ROWS = 256
B_SUB = 32


def _dot(a, b):
    return jax.lax.dot_general(a, b, (((1,), (0,)), ((), ())), preferred_element_type=F32)


def _dot_nt(a, b):
    return jax.lax.dot_general(a, b, (((1,), (1,)), ((), ())), preferred_element_type=F32)


def _iota(shape, dim):
    return jax.lax.broadcasted_iota(jnp.int32, shape, dim)


def _gate(x, gw):
    return jax.nn.sigmoid(jnp.sum(x * gw, axis=-1, keepdims=True))


def _kernel(x_hbm, mem0_ref, wq_hbm, wk_hbm, wv_hbm, wo_hbm, bqkv_hbm, bo_hbm, gw_ref,
            out_hbm,
            x_v, bqkv_v, bo_v, bqkv_p, bo_p, stage, w_all, wo_v, bq_s, bk_s, bv_s, bo_s, gb_s,
            o_s, out_v, sem_in, sem_w, sem_out, *, seg, dh):
    S, D = x_v.shape
    M = mem0_ref.shape[0]
    L = M + seg
    n_seg = S // seg
    PW = 2 * dh
    n_pair = wo_v.shape[0] // PW
    n_blk = S // B_ROWS
    ppb = n_pair // n_blk
    nc = D // LANES
    bdh = D // B_HEADS

    cp_bqkv = pltpu.make_async_copy(bqkv_hbm, bqkv_v, sem_in.at[0])
    cp_x = pltpu.make_async_copy(x_hbm, x_v, sem_in.at[1])
    cp_bo = pltpu.make_async_copy(bo_hbm, bo_v, sem_in.at[2])
    cp_wo = pltpu.make_async_copy(wo_hbm, wo_v, sem_in.at[3])

    def cp_w(j, i):
        rows = pl.ds(i * (ppb * PW), ppb * PW)
        return pltpu.make_async_copy((wq_hbm, wk_hbm, wv_hbm)[j].at[rows], stage.at[j, rows],
                                     sem_w.at[j, i])

    cp_bqkv.start()
    cp_bo.start()
    cp_x.start()
    r, c = _iota((D, D), 0), _iota((D, D), 1)
    perm = jnp.where(r == (c & (B_HEADS - 1)) * bdh + (c >> 5), 1.0, 0.0).astype(BF16)
    perm_t = jnp.where(c == (r & (B_HEADS - 1)) * bdh + (r >> 5), 1.0, 0.0).astype(BF16)
    cp_bqkv.wait()
    for i in range(n_blk):
        for j in range(3):
            cp_w(j, i).start()
    cp_wo.start()
    for j in range(3):
        bqkv_p[:, j * D:(j + 1) * D] = _dot(bqkv_v[:, j * D:(j + 1) * D], perm).astype(BF16)
    cp_bo.wait()
    bo_p[...] = _dot(perm_t, bo_v[...]).astype(BF16)
    cp_x.wait()

    gw = gw_ref[...].astype(F32)

    kv0 = _dot(x_v[0:16, :], bqkv_p[:, D:])[0:1]
    for cc in range(nc):
        bk_s[cc, 0:B_HALO, :] = jnp.broadcast_to(kv0[:, cc * LANES:(cc + 1) * LANES],
                                                 (B_HALO, LANES))
        bv_s[cc, 0:B_HALO, :] = jnp.broadcast_to(kv0[:, D + cc * LANES:D + (cc + 1) * LANES],
                                                 (B_HALO, LANES))

    def b_block(i, _):
        for j in range(3):
            cp_w(j, i).wait()
        r0 = pl.multiple_of(i * B_ROWS, B_ROWS)
        xb = x_v[pl.ds(r0, B_ROWS), :]
        bq_s[...] = _dot(xb, bqkv_p[:, 0:D]) * (bdh ** -0.5)
        for t, dst in ((1, bk_s), (2, bv_s)):
            y = _dot(xb, bqkv_p[:, t * D:(t + 1) * D])
            for cc in range(nc):
                dst[cc, pl.ds(r0 + B_HALO, B_ROWS), :] = y[:, cc * LANES:(cc + 1) * LANES]

        for u in range(ppb):
            p = i * ppb + u
            rows = pl.ds(pl.multiple_of(p * PW, PW), PW)
            for j in range(3):
                w_all[p, :, j * PW:(j + 1) * PW] = stage[j, rows, :].T

        for sb in range(B_ROWS // B_SUB):
            base = r0 + (B_HALO + sb * B_SUB)
            pos = r0 + sb * B_SUB + _iota((B_SUB, LANES), 0)
            q = [bq_s[sb * B_SUB:(sb + 1) * B_SUB, cc * LANES:(cc + 1) * LANES] for cc in range(nc)]
            logits = []
            for w in range(B_WIN):
                rows = pl.ds(base - w * B_DIL, B_SUB)
                t = q[0] * bk_s[0, rows, :]
                for cc in range(1, nc):
                    t = t + q[cc] * bk_s[cc, rows, :]
                t = t + pltpu.roll(t, 2 * B_HEADS, 1)
                t = t + pltpu.roll(t, B_HEADS, 1)
                if sb * B_SUB < w * B_DIL:
                    t = jnp.where(pos >= w * B_DIL, t, NEG)
                logits.append(t)
            mx = functools.reduce(jnp.maximum, logits)
            e = [jnp.exp(t - mx) for t in logits]
            inv = 1.0 / functools.reduce(jnp.add, e)
            for cc in range(nc):
                o = e[0] * bv_s[cc, pl.ds(base, B_SUB), :]
                for w in range(1, B_WIN):
                    o = o + e[w] * bv_s[cc, pl.ds(base - w * B_DIL, B_SUB), :]
                bo_s[sb * B_SUB:(sb + 1) * B_SUB, cc * LANES:(cc + 1) * LANES] = (
                    o * inv).astype(BF16)

        b = _dot(bo_s[...], bo_p[...])
        gb_s[pl.ds(r0, B_ROWS), :] = (1.0 - _gate(xb.astype(F32), gw)) * b
        return None

    jax.lax.fori_loop(0, n_blk, b_block, None)
    cp_wo.wait()

    row, lane = _iota((L, 2 * L), 0), _iota((L, 2 * L), 1)
    is_a = lane < L
    key = jnp.where(is_a, lane, lane - L)
    keep = (row < M) | (row >= key)
    lo_half = _iota((L, LANES), 1) < dh - LANES
    zeros = jnp.zeros((L, LANES), F32)
    scale = dh ** -0.5

    def split_heads(t):
        mid = t[:, LANES:2 * LANES]
        top = jnp.concatenate([t[:, :LANES], jnp.where(lo_half, mid, 0.0), zeros], axis=1)
        bot = jnp.concatenate([zeros, jnp.where(lo_half, 0.0, mid), t[:, 2 * LANES:]], axis=1)
        return jnp.concatenate([top, bot], axis=0).astype(BF16)

    def softmax(s):
        s = jnp.where(keep, s * scale, NEG)
        m_a = jnp.max(jnp.where(is_a, s, -jnp.inf), axis=1, keepdims=True)
        m_b = jnp.max(jnp.where(is_a, -jnp.inf, s), axis=1, keepdims=True)
        e = jnp.exp(s - jnp.where(is_a, m_a, m_b))
        l_a = jnp.sum(jnp.where(is_a, e, 0.0), axis=1, keepdims=True)
        l_b = jnp.sum(jnp.where(is_a, 0.0, e), axis=1, keepdims=True)
        return e / jnp.where(is_a, l_a, l_b)

    def cp_out(s):
        rows = pl.ds(pl.multiple_of(s * seg, seg), seg)
        return pltpu.make_async_copy(out_v.at[rows], out_hbm.at[rows], sem_out)

    def a_step(s, mem):
        rows = pl.ds(pl.multiple_of(s * seg, seg), seg)
        xs = x_v[rows, :].astype(F32)
        h = jnp.concatenate([mem, xs], axis=0)
        q, kb, vb, prob = {}, {}, {}, {}
        acc = []

        def st_qkv(p):
            q[p] = _dot(h, w_all[p, :, 0:PW])
            kb[p] = split_heads(_dot(h, w_all[p, :, PW:2 * PW]))
            vb[p] = split_heads(_dot(h, w_all[p, :, 2 * PW:3 * PW]))

        def st_score(p):
            prob[p] = softmax(_dot_nt(q.pop(p), kb.pop(p)))

        def st_pv(p):
            o_s[:, p * PW:(p + 1) * PW] = _dot(prob.pop(p), vb.pop(p))

        def st_out(p0, p1):
            t = _dot(o_s[:, p0 * PW:p1 * PW], wo_v[p0 * PW:p1 * PW, :])
            acc.append(t if not acc else acc.pop() + t)

        quarter = n_pair // 4
        for t in range(n_pair + 2):
            if t < n_pair:
                st_qkv(t)
            else:
                st_out((t - n_pair) * quarter, (t - n_pair + 1) * quarter)
            if t >= 2:
                st_pv(t - 2)
            if 1 <= t <= n_pair:
                st_score(t - 1)
        st_out(2 * quarter, n_pair)

        o = acc.pop()
        out_v[rows, :] = (_gate(xs, gw) * o[M:] + gb_s[rows, :]).astype(out_v.dtype)
        cp_out(s).start()
        return o[:M].astype(BF16).astype(F32)

    jax.lax.fori_loop(0, n_seg, a_step, mem0_ref[...].astype(F32))
    pltpu.make_async_copy(out_v, out_hbm, sem_out).wait()


@functools.partial(jax.jit, static_argnames=("A_seg_len",))
def pallas_gated_mix__memory_aug_recurrent_mem_tr__sliding_local_dilated__prompt_kernel(
    A_x, A_mem0, A_Wq, A_Wk, A_Wv, A_Wo, A_seg_len, B_x, B_wqkv, B_wo, gate_w,
):
    del B_x
    B, S, D = A_x.shape
    M = A_mem0.shape[1]
    H, dh = A_Wq.shape[1:]
    seg = int(A_seg_len)
    L = M + seg
    assert B == 1 and S % B_ROWS == 0 and S % seg == 0 and 2 * dh == 3 * LANES and 2 * L <= LANES
    n_pair, pw, nc = H // 2, 2 * dh, D // LANES

    def wt(w):
        return w.transpose(1, 2, 0).reshape(H * dh, D)

    hbm = pl.BlockSpec(memory_space=pl.ANY)
    vmem = pl.BlockSpec(memory_space=pltpu.VMEM)
    out = pl.pallas_call(
        functools.partial(_kernel, seg=seg, dh=dh),
        out_shape=jax.ShapeDtypeStruct((S, D), A_x.dtype),
        in_specs=[hbm, vmem, hbm, hbm, hbm, hbm, hbm, hbm, vmem],
        out_specs=hbm,
        scratch_shapes=[
            pltpu.VMEM((S, D), BF16),
            pltpu.VMEM((D, 3 * D), BF16),
            pltpu.VMEM((D, D), BF16),
            pltpu.VMEM((D, 3 * D), BF16),
            pltpu.VMEM((D, D), BF16),
            pltpu.VMEM((3, H * dh, D), BF16),
            pltpu.VMEM((n_pair, D, 3 * pw), BF16),
            pltpu.VMEM((H * dh, D), BF16),
            pltpu.VMEM((B_ROWS, D), F32),
            pltpu.VMEM((nc, B_HALO + S, LANES), F32),
            pltpu.VMEM((nc, B_HALO + S, LANES), F32),
            pltpu.VMEM((B_ROWS, D), BF16),
            pltpu.VMEM((S, D), F32),
            pltpu.VMEM((L, H * dh), F32),
            pltpu.VMEM((S, D), A_x.dtype),
            pltpu.SemaphoreType.DMA((4,)),
            pltpu.SemaphoreType.DMA((3, S // B_ROWS)),
            pltpu.SemaphoreType.DMA(()),
        ],
        compiler_params=pltpu.CompilerParams(vmem_limit_bytes=112 * 2**20),
    )(A_x.reshape(S, D), A_mem0.reshape(M, D), wt(A_Wq), wt(A_Wk), wt(A_Wv),
      A_Wo.reshape(H * dh, D), B_wqkv, B_wo, gate_w.reshape(1, D))
    return out.reshape(B, S, D)
```

```python
import functools

import jax
import jax.numpy as jnp
import jax.experimental.pallas as pl
import jax.experimental.pallas.tpu as pltpu

F32 = jnp.float32
BF16 = jnp.bfloat16
NEG = -1000000000.0
LANES = 128

B_HEADS, B_WIN, B_DIL = 32, 8, 2
B_HALO = 16
B_ROWS = 128
B_SUB = 32


def _dot(a, b):
    return jax.lax.dot_general(a, b, (((1,), (0,)), ((), ())), preferred_element_type=F32)


def _dot_nt(a, b):
    return jax.lax.dot_general(a, b, (((1,), (1,)), ((), ())), preferred_element_type=F32)


def _iota(shape, dim):
    return jax.lax.broadcasted_iota(jnp.int32, shape, dim)


def _tile(c):
    return slice(c * LANES, (c + 1) * LANES)


def _dot_tiles(a, w_ref, first, n):
    w = jnp.concatenate([w_ref[first + c] for c in range(n)], axis=1)
    return _dot(a, w if w.dtype == BF16 else pltpu.bitcast(w, BF16))


def _interleave(*gens):
    gens = list(gens)
    while gens:
        gens = [g for g in gens if next(g, StopIteration) is not StopIteration]


def _gate(x, gw):
    return jax.nn.sigmoid(jnp.sum(x * gw, axis=-1, keepdims=True))


def _kernel(x_hbm, mem0_ref, wq_hbm, wk_hbm, wv_hbm, wo_hbm, bqkv_hbm, bo_hbm, gw_ref,
            out_hbm,
            x_v, bqkv_v, bo_v, tmp_s, bqkv_p, bo_p, stage, w_all, wo_v, bq0, bk0, bv0, ba0, bq1, bk1, bv1, ba1, gb_s,
            o_s, out_v, sem_in, sem_b, sem_w, sem_out, *, seg, dh):
    S, D = x_v.shape
    M = mem0_ref.shape[0]
    L = M + seg
    n_seg = S // seg
    PW = 2 * dh
    n_pair = wo_v.shape[0] // PW
    n_blk = S // (2 * B_ROWS)
    ppb = n_pair // n_blk
    nc = D // LANES
    ntp = PW // LANES
    assert ppb == 2
    bdh = D // B_HEADS

    def cp_bqkv(i):
        rows = pl.ds(i * LANES, LANES)
        return pltpu.make_async_copy(bqkv_hbm.at[rows], bqkv_v.at[rows], sem_b.at[i])

    cp_x = pltpu.make_async_copy(x_hbm, x_v, sem_in.at[0])
    cp_bo = pltpu.make_async_copy(bo_hbm, bo_v, sem_in.at[1])

    def cp_w(j, i):
        rows = pl.ds(i * (ppb * PW), ppb * PW)
        return pltpu.make_async_copy((wq_hbm, wk_hbm, wv_hbm)[j].at[rows], stage.at[j, rows],
                                     sem_w.at[j, i])

    def cp_wo(i):
        rows = pl.ds(i * (ppb * PW), ppb * PW)
        return pltpu.make_async_copy(wo_hbm.at[rows], wo_v.at[rows], sem_w.at[3, i])

    def reorder_rows(dst, c, row0):
        for d in range(bdh):
            t = tmp_s[pl.ds(row0 + d, B_HEADS, stride=bdh), :]
            dst[c, row0 + d * B_HEADS:row0 + (d + 1) * B_HEADS, :] = t.astype(BF16)

    cp_bqkv(0).start()
    cp_bqkv(1).start()
    for i in range(nc):
        cp_bqkv(i).wait()
        if i + 2 < nc:
            cp_bqkv(i + 2).start()
        if i == 1:
            cp_x.start()
        if i == 3:
            cp_bo.start()
            for j in range(3):
                cp_w(j, 0).start()
        for j in range(3):
            tmp_s[j * D:(j + 1) * D, :] = bqkv_v[_tile(i), j * D:(j + 1) * D].astype(F32).T
            reorder_rows(bqkv_p, i, j * D)
    for j in range(3):
        cp_w(j, 1).start()
    cp_bo.wait()
    for cc in range(nc):
        tmp_s[0:D, :] = bo_v[:, _tile(cc)].astype(F32)
        reorder_rows(bo_p, cc, 0)
    cp_x.wait()

    gw = gw_ref[...].astype(F32)

    def b_proj(r0, buf, prev, first):
        q_s, k_s, v_s, _ = buf
        xb = x_v[pl.ds(r0, B_ROWS), :]

        def proj(t):
            return _dot_nt(xb, jnp.concatenate(
                [bqkv_p[c, t * D:(t + 1) * D, :] for c in range(nc)], axis=1))

        for t, dst, src in ((1, k_s, prev[1]), (2, v_s, prev[2])):
            y = proj(t)
            for cc in range(nc):
                yc = y[:, _tile(cc)]
                halo = src[cc, B_ROWS:, :]
                if first is not None:
                    halo = jnp.where(first, jnp.broadcast_to(yc[0:1], halo.shape), halo)
                dst[cc, :B_HALO, :] = halo
                dst[cc, B_HALO:, :] = yc
            yield
        q_s[...] = proj(0) * (bdh ** -0.5)
        yield

    def w_transpose(p):
        rows = pl.ds(pl.multiple_of(p * PW, PW), PW)
        for j in range(3):
            t = stage[j, rows, :].T
            for c in range(ntp):
                w_all[(p * 3 + j) * ntp + c] = pltpu.bitcast(t[:, _tile(c)], jnp.uint32)
            yield

    def b_attn(r0, buf, first):
        q_s, k_s, v_s, att_s = buf
        half = B_WIN // 2
        shift = half * B_DIL
        for sb in range(B_ROWS // B_SUB):
            base = B_HALO + sb * B_SUB
            out_rows = slice(sb * B_SUB, (sb + 1) * B_SUB)
            logits = [None] * B_WIN
            for cc in range(nc):
                q = q_s[out_rows, _tile(cc)]
                for w in range(half):
                    k = k_s[cc, pl.ds(base - w * B_DIL - shift, B_SUB + shift), :]
                    for ww, kk in ((w, k[shift:]), (w + half, k[:B_SUB])):
                        logits[ww] = q * kk if cc == 0 else logits[ww] + q * kk
            for w in range(B_WIN):
                t = logits[w]
                t = t + pltpu.roll(t, 2 * B_HEADS, 1)
                t = t + pltpu.roll(t, B_HEADS, 1)
                if first is not None and sb * B_SUB < w * B_DIL:
                    pos = r0 + sb * B_SUB + _iota((B_SUB, LANES), 0)
                    t = jnp.where(pos >= w * B_DIL, t, NEG)
                logits[w] = t
            mx = functools.reduce(jnp.maximum, logits)
            e = [jnp.exp(t - mx) for t in logits]
            inv = 1.0 / functools.reduce(jnp.add, e)
            for cc in range(nc):
                o = None
                for w in range(half):
                    v = v_s[cc, pl.ds(base - w * B_DIL - shift, B_SUB + shift), :]
                    t = e[w] * v[shift:] + e[w + half] * v[:B_SUB]
                    o = t if o is None else o + t
                att_s[out_rows, _tile(cc)] = (o * inv).astype(BF16)
            yield

    def b_out(r0, buf):
        rows = pl.ds(r0, B_ROWS)
        b = _dot_tiles(buf[3][...], bo_p, 0, nc)
        gb_s[rows, :] = (1.0 - _gate(x_v[rows, :].astype(F32), gw)) * b

    buf0, buf1 = (bq0, bk0, bv0, ba0), (bq1, bk1, bv1, ba1)
    for ref in (bq1, bk1, bv1):
        ref[...] = jnp.zeros(ref.shape, ref.dtype)

    def b_block(i, _):
        for j in range(3):
            cp_w(j, i).wait()

        @pl.when(i + 2 < n_blk)
        def _():
            for j in range(3):
                cp_w(j, i + 2).start()

        cp_wo(i).start()
        r0 = pl.multiple_of(i * (2 * B_ROWS), B_ROWS)
        r1 = pl.multiple_of(r0 + B_ROWS, B_ROWS)
        r_prev = pl.multiple_of(jnp.maximum(r0 - B_ROWS, 0), B_ROWS)
        _interleave(b_proj(r0, buf0, buf1, i == 0), b_attn(r_prev, buf1, None),
                    w_transpose(i * ppb))
        _interleave(b_proj(r1, buf1, buf0, None), b_attn(r0, buf0, i == 0),
                    w_transpose(i * ppb + 1))
        b_out(r_prev, buf1)
        b_out(r0, buf0)
        return None

    jax.lax.fori_loop(0, n_blk, b_block, None)
    _interleave(b_attn(S - B_ROWS, buf1, None))
    b_out(S - B_ROWS, buf1)
    for i in range(n_blk):
        cp_wo(i).wait()

    row, lane = _iota((L, 2 * L), 0), _iota((L, 2 * L), 1)
    is_a = lane < L
    key = jnp.where(is_a, lane, lane - L)
    keep = (row < M) | (row >= key)
    lo_half = _iota((L, LANES), 1) < dh - LANES
    zeros = jnp.zeros((L, LANES), F32)
    scale = dh ** -0.5

    def split_heads(t):
        mid = t[:, LANES:2 * LANES]
        top = jnp.concatenate([t[:, :LANES], jnp.where(lo_half, mid, 0.0), zeros], axis=1)
        bot = jnp.concatenate([zeros, jnp.where(lo_half, 0.0, mid), t[:, 2 * LANES:]], axis=1)
        return jnp.concatenate([top, bot], axis=0).astype(BF16)

    def softmax(s):
        s = jnp.where(keep, s * scale, NEG)
        m_a = jnp.max(jnp.where(is_a, s, -jnp.inf), axis=1, keepdims=True)
        m_b = jnp.max(jnp.where(is_a, -jnp.inf, s), axis=1, keepdims=True)
        e = jnp.exp(s - jnp.where(is_a, m_a, m_b))
        l_a = jnp.sum(jnp.where(is_a, e, 0.0), axis=1, keepdims=True)
        l_b = jnp.sum(jnp.where(is_a, 0.0, e), axis=1, keepdims=True)
        return e / jnp.where(is_a, l_a, l_b)

    def cp_out(s):
        rows = pl.ds(pl.multiple_of(s * seg, seg), seg)
        return pltpu.make_async_copy(out_v.at[rows], out_hbm.at[rows], sem_out)

    def a_step(s, mem):
        rows = pl.ds(pl.multiple_of(s * seg, seg), seg)
        xs = x_v[rows, :].astype(F32)
        h = jnp.concatenate([mem, xs], axis=0)
        q, kb, vb, prob = {}, {}, {}, {}
        acc = []

        def st_qkv(p):
            q[p] = _dot_tiles(h, w_all, 3 * p * ntp, ntp)
            kb[p] = split_heads(_dot_tiles(h, w_all, (3 * p + 1) * ntp, ntp))
            vb[p] = split_heads(_dot_tiles(h, w_all, (3 * p + 2) * ntp, ntp))

        def st_score(p):
            prob[p] = softmax(_dot_nt(q.pop(p), kb.pop(p)))

        def st_pv(p):
            o_s[:, p * PW:(p + 1) * PW] = _dot(prob.pop(p), vb.pop(p))

        def st_out(p0, p1):
            t = _dot(o_s[:, p0 * PW:p1 * PW], wo_v[p0 * PW:p1 * PW, :])
            acc.append(t if not acc else acc.pop() + t)

        quarter = n_pair // 4
        for t in range(n_pair + 2):
            if t < n_pair:
                st_qkv(t)
            else:
                st_out((t - n_pair) * quarter, (t - n_pair + 1) * quarter)
            if t >= 2:
                st_pv(t - 2)
            if 1 <= t <= n_pair:
                st_score(t - 1)
        st_out(2 * quarter, n_pair)

        o = acc.pop()
        out_v[rows, :] = (_gate(xs, gw) * o[M:] + gb_s[rows, :]).astype(out_v.dtype)
        cp_out(s).start()
        return o[:M].astype(BF16).astype(F32)

    jax.lax.fori_loop(0, n_seg, a_step, mem0_ref[...].astype(F32))
    pltpu.make_async_copy(out_v, out_hbm, sem_out).wait()


@functools.partial(jax.jit, static_argnames=("A_seg_len",))
def pallas_gated_mix__memory_aug_recurrent_mem_tr__sliding_local_dilated__prompt_kernel(
    A_x, A_mem0, A_Wq, A_Wk, A_Wv, A_Wo, A_seg_len, B_x, B_wqkv, B_wo, gate_w,
):
    del B_x
    B, S, D = A_x.shape
    M = A_mem0.shape[1]
    H, dh = A_Wq.shape[1:]
    seg = int(A_seg_len)
    L = M + seg
    assert B == 1 and S % (2 * B_ROWS) == 0 and S % seg == 0 and 2 * dh == 3 * LANES and 2 * L <= LANES
    nc = D // LANES

    def wt(w):
        return w.transpose(1, 2, 0).reshape(H * dh, D)

    hbm = pl.BlockSpec(memory_space=pl.ANY)
    vmem = pl.BlockSpec(memory_space=pltpu.VMEM)
    out = pl.pallas_call(
        functools.partial(_kernel, seg=seg, dh=dh),
        out_shape=jax.ShapeDtypeStruct((S, D), A_x.dtype),
        in_specs=[hbm, vmem, hbm, hbm, hbm, hbm, hbm, hbm, vmem],
        out_specs=hbm,
        scratch_shapes=[
            pltpu.VMEM((S, D), BF16),
            pltpu.VMEM((D, 3 * D), BF16),
            pltpu.VMEM((D, D), BF16),
            pltpu.VMEM((3 * D, LANES), F32),
            pltpu.VMEM((nc, 3 * D, LANES), BF16),
            pltpu.VMEM((nc, D, LANES), BF16),
            pltpu.VMEM((3, H * dh, D), BF16),
            pltpu.VMEM((3 * H * dh // LANES, D // 2, LANES), jnp.uint32),
            pltpu.VMEM((H * dh, D), BF16),
            *[pltpu.VMEM((B_ROWS, D), F32),
              pltpu.VMEM((nc, B_HALO + B_ROWS, LANES), F32),
              pltpu.VMEM((nc, B_HALO + B_ROWS, LANES), F32),
              pltpu.VMEM((B_ROWS, D), BF16)] * 2,
            pltpu.VMEM((S, D), F32),
            pltpu.VMEM((L, H * dh), F32),
            pltpu.VMEM((S, D), A_x.dtype),
            pltpu.SemaphoreType.DMA((2,)),
            pltpu.SemaphoreType.DMA((nc,)),
            pltpu.SemaphoreType.DMA((4, S // (2 * B_ROWS))),
            pltpu.SemaphoreType.DMA(()),
        ],
        compiler_params=pltpu.CompilerParams(vmem_limit_bytes=112 * 2**20),
    )(A_x.reshape(S, D), A_mem0.reshape(M, D), wt(A_Wq), wt(A_Wk), wt(A_Wv),
      A_Wo.reshape(H * dh, D), B_wqkv, B_wo, gate_w.reshape(1, D))
    return out.reshape(B, S, D)
```

```python
import functools

import jax
import jax.numpy as jnp
import jax.experimental.pallas as pl
import jax.experimental.pallas.tpu as pltpu

F32 = jnp.float32
BF16 = jnp.bfloat16
NEG = -1000000000.0
LANES = 128

B_HEADS, B_WIN, B_DIL = 32, 8, 2
B_HALO = 16
B_ROWS = 128
B_SUB = 32
V_LAG, O_LAG = 3, 4
A_UNROLL = 2


def _dot(a, b):
    return jax.lax.dot_general(a, b, (((1,), (0,)), ((), ())), preferred_element_type=F32)


def _dot_nt(a, b):
    return jax.lax.dot_general(a, b, (((1,), (1,)), ((), ())), preferred_element_type=F32)


def _iota(shape, dim):
    return jax.lax.broadcasted_iota(jnp.int32, shape, dim)


def _tile(c):
    return slice(c * LANES, (c + 1) * LANES)


def _dot_tiles(a, w_ref, first, n):
    w = jnp.concatenate([w_ref[first + c] for c in range(n)], axis=1)
    return _dot(a, w if w.dtype == BF16 else pltpu.bitcast(w, BF16))


def _interleave(*gens):
    gens = list(gens)
    while gens:
        gens = [g for g in gens if next(g, StopIteration) is not StopIteration]


def _gate(x, gw):
    return jax.nn.sigmoid(jnp.sum(x * gw, axis=-1, keepdims=True))


def _kernel(x_hbm, mem0_ref, wq_hbm, wk_hbm, wv_hbm, wo_hbm, bqkv_hbm, bo_hbm, gw_ref,
            out_hbm,
            x_v, bqkv_v, bo_v, tmp_s, bqkv_p, bo_p, stage, w_all, wo_v, bq0, bk0, bv0, ba0, bq1, bk1, bv1, ba1, gb_s,
            out_v, sem_in, sem_b, sem_w, sem_out, *, seg, dh):
    S, D = x_v.shape
    M = mem0_ref.shape[0]
    L = M + seg
    n_seg = S // seg
    PW = 2 * dh
    n_pair = wo_v.shape[0] // PW
    n_blk = S // (2 * B_ROWS)
    ppb = n_pair // n_blk
    nc = D // LANES
    ntp = PW // LANES
    assert ppb == 2
    bdh = D // B_HEADS

    def cp_bqkv(i):
        rows = pl.ds(i * LANES, LANES)
        return pltpu.make_async_copy(bqkv_hbm.at[rows], bqkv_v.at[rows], sem_b.at[i])

    cp_x = pltpu.make_async_copy(x_hbm, x_v, sem_in.at[0])
    cp_bo = pltpu.make_async_copy(bo_hbm, bo_v, sem_in.at[1])

    def cp_w(j, i):
        rows = pl.ds(i * (ppb * PW), ppb * PW)
        return pltpu.make_async_copy((wq_hbm, wk_hbm, wv_hbm)[j].at[rows], stage.at[j, rows],
                                     sem_w.at[j, i])

    def cp_wo(i):
        rows = pl.ds(i * (ppb * PW), ppb * PW)
        return pltpu.make_async_copy(wo_hbm.at[rows], wo_v.at[rows], sem_w.at[3, i])

    def reorder_rows(dst, c, row0):
        for d in range(bdh):
            t = tmp_s[pl.ds(row0 + d, B_HEADS, stride=bdh), :]
            dst[c, row0 + d * B_HEADS:row0 + (d + 1) * B_HEADS, :] = t.astype(BF16)

    cp_bqkv(0).start()
    cp_bqkv(1).start()
    for i in range(nc):
        cp_bqkv(i).wait()
        if i + 2 < nc:
            cp_bqkv(i + 2).start()
        if i == 1:
            cp_x.start()
        if i == 3:
            cp_bo.start()
            for j in range(3):
                cp_w(j, 0).start()
        for j in range(3):
            tmp_s[j * D:(j + 1) * D, :] = bqkv_v[_tile(i), j * D:(j + 1) * D].astype(F32).T
            reorder_rows(bqkv_p, i, j * D)
    for j in range(3):
        cp_w(j, 1).start()
    cp_bo.wait()
    for cc in range(nc):
        tmp_s[0:D, :] = bo_v[:, _tile(cc)].astype(F32)
        reorder_rows(bo_p, cc, 0)
    cp_x.wait()

    gw = gw_ref[...].astype(F32)

    def b_proj(r0, buf, prev, first):
        q_s, k_s, v_s, _ = buf
        xb = x_v[pl.ds(r0, B_ROWS), :]

        def proj(t):
            return _dot_nt(xb, jnp.concatenate(
                [bqkv_p[c, t * D:(t + 1) * D, :] for c in range(nc)], axis=1))

        for t, dst, src in ((1, k_s, prev[1]), (2, v_s, prev[2])):
            y = proj(t)
            for cc in range(nc):
                yc = y[:, _tile(cc)]
                halo = src[cc, B_ROWS:, :]
                if first is not None:
                    halo = jnp.where(first, jnp.broadcast_to(yc[0:1], halo.shape), halo)
                dst[cc, :B_HALO, :] = halo
                dst[cc, B_HALO:, :] = yc
            yield
        q_s[...] = proj(0) * (bdh ** -0.5)
        yield

    def w_transpose(p):
        rows = pl.ds(pl.multiple_of(p * PW, PW), PW)
        for j in range(3):
            t = stage[j, rows, :].T
            for c in range(ntp):
                w_all[(p * 3 + j) * ntp + c] = pltpu.bitcast(t[:, _tile(c)], jnp.uint32)
            yield

    def b_attn(r0, buf, first):
        q_s, k_s, v_s, att_s = buf
        half = B_WIN // 2
        shift = half * B_DIL
        for sb in range(B_ROWS // B_SUB):
            base = B_HALO + sb * B_SUB
            out_rows = slice(sb * B_SUB, (sb + 1) * B_SUB)
            logits = [None] * B_WIN
            for cc in range(nc):
                q = q_s[out_rows, _tile(cc)]
                for w in range(half):
                    k = k_s[cc, pl.ds(base - w * B_DIL - shift, B_SUB + shift), :]
                    for ww, kk in ((w, k[shift:]), (w + half, k[:B_SUB])):
                        logits[ww] = q * kk if cc == 0 else logits[ww] + q * kk
            for w in range(B_WIN):
                t = logits[w]
                t = t + pltpu.roll(t, 2 * B_HEADS, 1)
                t = t + pltpu.roll(t, B_HEADS, 1)
                if first is not None and sb * B_SUB < w * B_DIL:
                    pos = r0 + sb * B_SUB + _iota((B_SUB, LANES), 0)
                    t = jnp.where(pos >= w * B_DIL, t, NEG)
                logits[w] = t
            mx = functools.reduce(jnp.maximum, logits)
            e = [jnp.exp(t - mx) for t in logits]
            inv = 1.0 / functools.reduce(jnp.add, e)
            for cc in range(nc):
                o = None
                for w in range(half):
                    v = v_s[cc, pl.ds(base - w * B_DIL - shift, B_SUB + shift), :]
                    t = e[w] * v[shift:] + e[w + half] * v[:B_SUB]
                    o = t if o is None else o + t
                att_s[out_rows, _tile(cc)] = (o * inv).astype(BF16)
            yield

    def b_out(r0, buf):
        rows = pl.ds(r0, B_ROWS)
        b = _dot_tiles(buf[3][...], bo_p, 0, nc)
        gb_s[rows, :] = (1.0 - _gate(x_v[rows, :].astype(F32), gw)) * b

    buf0, buf1 = (bq0, bk0, bv0, ba0), (bq1, bk1, bv1, ba1)
    for ref in (bq1, bk1, bv1):
        ref[...] = jnp.zeros(ref.shape, ref.dtype)

    def b_block(i, _):
        for j in range(3):
            cp_w(j, i).wait()

        @pl.when(i + 2 < n_blk)
        def _():
            for j in range(3):
                cp_w(j, i + 2).start()

        cp_wo(i).start()
        r0 = pl.multiple_of(i * (2 * B_ROWS), B_ROWS)
        r1 = pl.multiple_of(r0 + B_ROWS, B_ROWS)
        r_prev = pl.multiple_of(jnp.maximum(r0 - B_ROWS, 0), B_ROWS)
        _interleave(b_proj(r0, buf0, buf1, i == 0), b_attn(r_prev, buf1, None),
                    w_transpose(i * ppb))
        _interleave(b_proj(r1, buf1, buf0, None), b_attn(r0, buf0, i == 0),
                    w_transpose(i * ppb + 1))
        b_out(r_prev, buf1)
        b_out(r0, buf0)
        return None

    jax.lax.fori_loop(0, n_blk, b_block, None)
    _interleave(b_attn(S - B_ROWS, buf1, None))
    b_out(S - B_ROWS, buf1)
    for i in range(n_blk):
        cp_wo(i).wait()

    row, lane = _iota((L, 2 * L), 0), _iota((L, 2 * L), 1)
    is_a = lane < L
    key = jnp.where(is_a, lane, lane - L)
    keep = (row < M) | (row >= key)
    lo_half = _iota((L, LANES), 1) < dh - LANES
    zeros = jnp.zeros((L, LANES), F32)
    scale = dh ** -0.5

    def split_heads(t):
        mid = t[:, LANES:2 * LANES]
        top = jnp.concatenate([t[:, :LANES], jnp.where(lo_half, mid, 0.0), zeros], axis=1)
        bot = jnp.concatenate([zeros, jnp.where(lo_half, 0.0, mid), t[:, 2 * LANES:]], axis=1)
        return jnp.concatenate([top, bot], axis=0).astype(BF16)

    def softmax(s):
        s = jnp.where(keep, s * scale, NEG)
        m_a = jnp.max(jnp.where(is_a, s, -jnp.inf), axis=1, keepdims=True)
        m_b = jnp.max(jnp.where(is_a, -jnp.inf, s), axis=1, keepdims=True)
        e = jnp.exp(s - jnp.where(is_a, m_a, m_b))
        l_a = jnp.sum(jnp.where(is_a, e, 0.0), axis=1, keepdims=True)
        l_b = jnp.sum(jnp.where(is_a, 0.0, e), axis=1, keepdims=True)
        return e / jnp.where(is_a, l_a, l_b)

    def a_step(s, mem):
        rows = pl.ds(pl.multiple_of(s * seg, seg), seg)
        xs = x_v[rows, :].astype(F32)
        h = jnp.concatenate([mem, xs], axis=0)
        q, kb, vb, prob, att = {}, {}, {}, {}, {}
        acc = None
        for t in range(n_pair + V_LAG + 1):
            if t < n_pair:
                q[t] = _dot_tiles(h, w_all, 3 * t * ntp, ntp)
                kb[t] = split_heads(_dot_tiles(h, w_all, (3 * t + 1) * ntp, ntp))
            p = t - V_LAG
            if 0 <= p < n_pair:
                vb[p] = split_heads(_dot_tiles(h, w_all, (3 * p + 2) * ntp, ntp))
            p = t - 1
            if 0 <= p < n_pair:
                prob[p] = softmax(_dot_nt(q.pop(p), kb.pop(p)))
            p = t - V_LAG - 1 - O_LAG
            if p >= 0:
                y = _dot(att.pop(p), wo_v[p * PW:(p + 1) * PW, :])
                acc = y if acc is None else acc + y
            p = t - V_LAG - 1
            if p >= 0:
                att[p] = _dot(prob.pop(p), vb.pop(p))
        rest = jnp.concatenate([att[p] for p in sorted(att)], axis=1)
        o = jnp.concatenate(
            [acc[:, _tile(c)] + _dot(rest, wo_v[(n_pair - O_LAG) * PW:, _tile(c)])
             for c in range(nc)], axis=1)
        out_v[rows, :] = (_gate(xs, gw) * o[M:] + gb_s[rows, :]).astype(out_v.dtype)
        return o[:M].astype(BF16).astype(F32)

    def a_group(g, mem):
        for u in range(A_UNROLL):
            mem = a_step(g * A_UNROLL + u, mem)
        rows = pl.ds(pl.multiple_of(g * (A_UNROLL * seg), seg), A_UNROLL * seg)
        pltpu.make_async_copy(out_v.at[rows], out_hbm.at[rows], sem_out).start()
        return mem

    jax.lax.fori_loop(0, n_seg // A_UNROLL, a_group, mem0_ref[...].astype(F32))
    pltpu.make_async_copy(out_v, out_hbm, sem_out).wait()


@functools.partial(jax.jit, static_argnames=("A_seg_len",))
def pallas_gated_mix__memory_aug_recurrent_mem_tr__sliding_local_dilated__prompt_kernel(
    A_x, A_mem0, A_Wq, A_Wk, A_Wv, A_Wo, A_seg_len, B_x, B_wqkv, B_wo, gate_w,
):
    del B_x
    B, S, D = A_x.shape
    M = A_mem0.shape[1]
    H, dh = A_Wq.shape[1:]
    seg = int(A_seg_len)
    L = M + seg
    assert B == 1 and S % (2 * B_ROWS) == 0 and S % seg == 0 and 2 * dh == 3 * LANES and 2 * L <= LANES
    nc = D // LANES

    def wt(w):
        return w.transpose(1, 2, 0).reshape(H * dh, D)

    hbm = pl.BlockSpec(memory_space=pl.ANY)
    vmem = pl.BlockSpec(memory_space=pltpu.VMEM)
    out = pl.pallas_call(
        functools.partial(_kernel, seg=seg, dh=dh),
        out_shape=jax.ShapeDtypeStruct((S, D), A_x.dtype),
        in_specs=[hbm, vmem, hbm, hbm, hbm, hbm, hbm, hbm, vmem],
        out_specs=hbm,
        scratch_shapes=[
            pltpu.VMEM((S, D), BF16),
            pltpu.VMEM((D, 3 * D), BF16),
            pltpu.VMEM((D, D), BF16),
            pltpu.VMEM((3 * D, LANES), F32),
            pltpu.VMEM((nc, 3 * D, LANES), BF16),
            pltpu.VMEM((nc, D, LANES), BF16),
            pltpu.VMEM((3, H * dh, D), BF16),
            pltpu.VMEM((3 * H * dh // LANES, D // 2, LANES), jnp.uint32),
            pltpu.VMEM((H * dh, D), BF16),
            *[pltpu.VMEM((B_ROWS, D), F32),
              pltpu.VMEM((nc, B_HALO + B_ROWS, LANES), F32),
              pltpu.VMEM((nc, B_HALO + B_ROWS, LANES), F32),
              pltpu.VMEM((B_ROWS, D), BF16)] * 2,
            pltpu.VMEM((S, D), F32),
            pltpu.VMEM((S, D), A_x.dtype),
            pltpu.SemaphoreType.DMA((2,)),
            pltpu.SemaphoreType.DMA((nc,)),
            pltpu.SemaphoreType.DMA((4, S // (2 * B_ROWS))),
            pltpu.SemaphoreType.DMA(()),
        ],
        compiler_params=pltpu.CompilerParams(vmem_limit_bytes=112 * 2**20),
    )(A_x.reshape(S, D), A_mem0.reshape(M, D), wt(A_Wq), wt(A_Wk), wt(A_Wv),
      A_Wo.reshape(H * dh, D), B_wqkv, B_wo, gate_w.reshape(1, D))
    return out.reshape(B, S, D)
```

```python
import functools

import jax
import jax.numpy as jnp
import jax.experimental.pallas as pl
import jax.experimental.pallas.tpu as pltpu

F32 = jnp.float32
BF16 = jnp.bfloat16
NEG = -1000000000.0
LANES = 128

B_HEADS, B_WIN, B_DIL = 32, 8, 2
B_HALO = 16
B_ROWS = 128
B_SUB = 32
V_LAG, O_LAG = 3, 4
A_UNROLL = 3


def _dot(a, b):
    return jax.lax.dot_general(a, b, (((1,), (0,)), ((), ())), preferred_element_type=F32)


def _dot_nt(a, b):
    return jax.lax.dot_general(a, b, (((1,), (1,)), ((), ())), preferred_element_type=F32)


def _iota(shape, dim):
    return jax.lax.broadcasted_iota(jnp.int32, shape, dim)


def _tile(c):
    return slice(c * LANES, (c + 1) * LANES)


def _dot_tiles(a, w_ref, first, n):
    w = jnp.concatenate([w_ref[first + c] for c in range(n)], axis=1)
    return _dot(a, w if w.dtype == BF16 else pltpu.bitcast(w, BF16))


def _interleave(*gens):
    gens = list(gens)
    while gens:
        gens = [g for g in gens if next(g, StopIteration) is not StopIteration]


def _gate(x, gw):
    return jax.nn.sigmoid(jnp.sum(x * gw, axis=-1, keepdims=True))


def _kernel(x_hbm, mem0_ref, wq_hbm, wk_hbm, wv_hbm, wo_hbm, bqkv_hbm, bo_hbm, gw_ref,
            out_hbm,
            x_v, bqkv_v, bo_v, tmp_s, bqkv_p, bo_p, stage, w_all, wo_v, bq0, bk0, bv0, ba0, bq1, bk1, bv1, ba1, gb_s,
            out_v, sem_o, sem_b, sem_w, sem_out, *, seg, dh):
    S, D = x_v.shape
    M = mem0_ref.shape[0]
    L = M + seg
    n_seg = S // seg
    PW = 2 * dh
    n_pair = wo_v.shape[0] // PW
    n_blk = S // (2 * B_ROWS)
    ppb = n_pair // n_blk
    nc = D // LANES
    ntp = PW // LANES
    assert ppb == 2
    bdh = D // B_HEADS

    def cp_bqkv(i):
        rows = pl.ds(i * LANES, LANES)
        return pltpu.make_async_copy(bqkv_hbm.at[rows], bqkv_v.at[rows], sem_b.at[i])

    cp_bo = pltpu.make_async_copy(bo_hbm, bo_v, sem_b.at[nc])

    def cp_x(i):
        rows = pl.ds(i * (2 * B_ROWS), 2 * B_ROWS)
        return pltpu.make_async_copy(x_hbm.at[rows], x_v.at[rows], sem_w.at[3, i])

    def cp_w(j, i):
        n = ppb * PW
        return pltpu.make_async_copy((wq_hbm, wk_hbm, wv_hbm)[j].at[pl.ds(i * n, n)],
                                     stage.at[j, pl.ds((i + 1) * n, n)], sem_w.at[j, i])

    def cp_wo(i):
        rows = pl.ds(i * (n_pair * dh), n_pair * dh)
        return pltpu.make_async_copy(wo_hbm.at[rows], wo_v.at[rows], sem_o.at[i])

    def reorder_rows(dst, c, row0):
        for d in range(bdh):
            t = tmp_s[pl.ds(row0 + d, B_HEADS, stride=bdh), :]
            dst[c, row0 + d * B_HEADS:row0 + (d + 1) * B_HEADS, :] = t.astype(BF16)

    buf0, buf1 = (bq0, bk0, bv0, ba0), (bq1, bk1, bv1, ba1)
    cp_bqkv(0).start()
    cp_bqkv(1).start()
    for ref in (bq1, bk1, bv1):
        ref[...] = jnp.zeros(ref.shape, ref.dtype)
    stage[:, :ppb * PW, :] = jnp.zeros((3, ppb * PW, D), BF16)
    for i in range(nc):
        cp_bqkv(i).wait()
        if i + 2 < nc:
            cp_bqkv(i + 2).start()
        if i == 3:
            cp_x(0).start()
            cp_bo.start()
        if i == 4:
            cp_x(1).start()
            for j in range(3):
                cp_w(j, 0).start()
        for j in range(3):
            tmp_s[j * D:(j + 1) * D, :] = bqkv_v[_tile(i), j * D:(j + 1) * D].astype(F32).T
            reorder_rows(bqkv_p, i, j * D)
    cp_bo.wait()
    for cc in range(nc):
        tmp_s[0:D, :] = bo_v[:, _tile(cc)].astype(F32)
        reorder_rows(bo_p, cc, 0)

    gw = gw_ref[...].astype(F32)

    def b_proj(r0, buf, prev, first):
        q_s, k_s, v_s, _ = buf
        xb = x_v[pl.ds(r0, B_ROWS), :]

        def proj(t):
            return _dot_nt(xb, jnp.concatenate(
                [bqkv_p[c, t * D:(t + 1) * D, :] for c in range(nc)], axis=1))

        for t, dst, src in ((1, k_s, prev[1]), (2, v_s, prev[2])):
            y = proj(t)
            for cc in range(nc):
                yc = y[:, _tile(cc)]
                halo = src[cc, B_ROWS:, :]
                if first is not None:
                    halo = jnp.where(first, jnp.broadcast_to(yc[0:1], halo.shape), halo)
                dst[cc, :B_HALO, :] = halo
                dst[cc, B_HALO:, :] = yc
            yield
        q_s[...] = proj(0) * (bdh ** -0.5)
        yield

    def w_transpose(p):
        rows = pl.ds(pl.multiple_of((p + ppb) * PW, PW), PW)
        for j in range(3):
            t = stage[j, rows, :].T
            for c in range(ntp):
                w_all[(jnp.maximum(p, 0) * 3 + j) * ntp + c] = pltpu.bitcast(t[:, _tile(c)], jnp.uint32)
            yield

    def b_attn(r0, buf, first):
        q_s, k_s, v_s, att_s = buf
        half = B_WIN // 2
        shift = half * B_DIL
        for sb in range(B_ROWS // B_SUB):
            base = B_HALO + sb * B_SUB
            out_rows = slice(sb * B_SUB, (sb + 1) * B_SUB)
            logits = [None] * B_WIN
            for cc in range(nc):
                q = q_s[out_rows, _tile(cc)]
                for w in range(half):
                    k = k_s[cc, pl.ds(base - w * B_DIL - shift, B_SUB + shift), :]
                    for ww, kk in ((w, k[shift:]), (w + half, k[:B_SUB])):
                        logits[ww] = q * kk if cc == 0 else logits[ww] + q * kk
            for w in range(B_WIN):
                t = logits[w]
                t = t + pltpu.roll(t, 2 * B_HEADS, 1)
                t = t + pltpu.roll(t, B_HEADS, 1)
                if first is not None and sb * B_SUB < w * B_DIL:
                    pos = r0 + sb * B_SUB + _iota((B_SUB, LANES), 0)
                    t = jnp.where(pos >= w * B_DIL, t, NEG)
                logits[w] = t
            mx = functools.reduce(jnp.maximum, logits)
            e = [jnp.exp(t - mx) for t in logits]
            inv = 1.0 / functools.reduce(jnp.add, e)
            for cc in range(nc):
                o = None
                for w in range(half):
                    v = v_s[cc, pl.ds(base - w * B_DIL - shift, B_SUB + shift), :]
                    t = e[w] * v[shift:] + e[w + half] * v[:B_SUB]
                    o = t if o is None else o + t
                att_s[out_rows, _tile(cc)] = (o * inv).astype(BF16)
            yield

    def b_out(r0, buf):
        rows = pl.ds(r0, B_ROWS)
        b = _dot_tiles(buf[3][...], bo_p, 0, nc)
        gb_s[rows, :] = (1.0 - _gate(x_v[rows, :].astype(F32), gw)) * b

    def b_block(i, _):
        @pl.when(i + 2 < n_blk)
        def _():
            cp_x(i + 2).start()

        @pl.when(i + 1 < n_blk)
        def _():
            for j in range(3):
                cp_w(j, i + 1).start()

        @pl.when(i + 2 >= n_blk)
        def _():
            cp_wo(i + 2 - n_blk).start()

        @pl.when(i > 0)
        def _():
            for j in range(3):
                cp_w(j, i - 1).wait()

        cp_x(i).wait()
        r0 = pl.multiple_of(i * (2 * B_ROWS), B_ROWS)
        r1 = pl.multiple_of(r0 + B_ROWS, B_ROWS)
        r_prev = pl.multiple_of(jnp.maximum(r0 - B_ROWS, 0), B_ROWS)
        _interleave(b_proj(r0, buf0, buf1, i == 0), b_attn(r_prev, buf1, None),
                    w_transpose((i - 1) * ppb))
        _interleave(b_proj(r1, buf1, buf0, None), b_attn(r0, buf0, i == 0),
                    w_transpose((i - 1) * ppb + 1))
        b_out(r_prev, buf1)
        b_out(r0, buf0)
        return None

    jax.lax.fori_loop(0, n_blk, b_block, None)
    for j in range(3):
        cp_w(j, n_blk - 1).wait()
    _interleave(b_attn(S - B_ROWS, buf1, None), w_transpose(n_pair - 2), w_transpose(n_pair - 1))
    b_out(S - B_ROWS, buf1)

    row, lane = _iota((L, 2 * L), 0), _iota((L, 2 * L), 1)
    is_a = lane < L
    key = jnp.where(is_a, lane, lane - L)
    keep = (row < M) | (row >= key)
    lo_half = _iota((L, LANES), 1) < dh - LANES
    zeros = jnp.zeros((L, LANES), F32)
    scale = dh ** -0.5

    def split_heads(t):
        mid = t[:, LANES:2 * LANES]
        top = jnp.concatenate([t[:, :LANES], jnp.where(lo_half, mid, 0.0), zeros], axis=1)
        bot = jnp.concatenate([zeros, jnp.where(lo_half, 0.0, mid), t[:, 2 * LANES:]], axis=1)
        return jnp.concatenate([top, bot], axis=0).astype(BF16)

    def softmax(s):
        s = jnp.where(keep, s * scale, NEG)
        m_a = jnp.max(jnp.where(is_a, s, -jnp.inf), axis=1, keepdims=True)
        m_b = jnp.max(jnp.where(is_a, -jnp.inf, s), axis=1, keepdims=True)
        e = jnp.exp(s - jnp.where(is_a, m_a, m_b))
        l_a = jnp.sum(jnp.where(is_a, e, 0.0), axis=1, keepdims=True)
        l_b = jnp.sum(jnp.where(is_a, 0.0, e), axis=1, keepdims=True)
        return e / jnp.where(is_a, l_a, l_b)

    def a_step(s, mem, o_lag=O_LAG, before_out=lambda: None):
        rows = pl.ds(pl.multiple_of(s * seg, seg), seg)
        xs = x_v[rows, :].astype(F32)
        h = jnp.concatenate([mem, xs], axis=0)
        q, kb, vb, prob, att = {}, {}, {}, {}, {}
        acc = None
        for t in range(n_pair + V_LAG + 1):
            if t < n_pair:
                q[t] = _dot_tiles(h, w_all, 3 * t * ntp, ntp)
                kb[t] = split_heads(_dot_tiles(h, w_all, (3 * t + 1) * ntp, ntp))
            p = t - V_LAG
            if 0 <= p < n_pair:
                vb[p] = split_heads(_dot_tiles(h, w_all, (3 * p + 2) * ntp, ntp))
            p = t - 1
            if 0 <= p < n_pair:
                prob[p] = softmax(_dot_nt(q.pop(p), kb.pop(p)))
            p = t - V_LAG - 1 - o_lag
            if p >= 0:
                y = _dot(att.pop(p), wo_v[p * PW:(p + 1) * PW, :])
                acc = y if acc is None else acc + y
            p = t - V_LAG - 1
            if p >= 0:
                att[p] = _dot(prob.pop(p), vb.pop(p))
        before_out()
        rest = jnp.concatenate([att[p] for p in sorted(att)], axis=1)
        o = jnp.concatenate(
            [_dot(rest, wo_v[(n_pair - o_lag) * PW:, _tile(c)]) for c in range(nc)], axis=1)
        o = o if acc is None else acc + o
        out_v[rows, :] = (_gate(xs, gw) * o[M:] + gb_s[rows, :]).astype(out_v.dtype)
        return o[:M].astype(BF16).astype(F32)

    def store_out(s, n):
        rows = pl.ds(pl.multiple_of(s * seg, seg), n * seg)
        pltpu.make_async_copy(out_v.at[rows], out_hbm.at[rows], sem_out).start()

    def a_group(g, mem):
        s0 = 1 + g * A_UNROLL
        for u in range(A_UNROLL):
            mem = a_step(s0 + u, mem)
        store_out(s0, A_UNROLL)
        return mem

    def wait_wo():
        cp_wo(0).wait()
        cp_wo(1).wait()

    mem = a_step(0, mem0_ref[...].astype(F32), n_pair, wait_wo)
    store_out(0, 1)
    assert (n_seg - 1) % A_UNROLL == 0
    jax.lax.fori_loop(0, (n_seg - 1) // A_UNROLL, a_group, mem)
    pltpu.make_async_copy(out_v, out_hbm, sem_out).wait()


@functools.partial(jax.jit, static_argnames=("A_seg_len",))
def pallas_gated_mix__memory_aug_recurrent_mem_tr__sliding_local_dilated__prompt_kernel(
    A_x, A_mem0, A_Wq, A_Wk, A_Wv, A_Wo, A_seg_len, B_x, B_wqkv, B_wo, gate_w,
):
    del B_x
    B, S, D = A_x.shape
    M = A_mem0.shape[1]
    H, dh = A_Wq.shape[1:]
    seg = int(A_seg_len)
    L = M + seg
    assert B == 1 and S % (2 * B_ROWS) == 0 and S % seg == 0 and 2 * dh == 3 * LANES and 2 * L <= LANES
    nc = D // LANES

    def wt(w):
        return w.transpose(1, 2, 0).reshape(H * dh, D)

    hbm = pl.BlockSpec(memory_space=pl.ANY)
    vmem = pl.BlockSpec(memory_space=pltpu.VMEM)
    out = pl.pallas_call(
        functools.partial(_kernel, seg=seg, dh=dh),
        out_shape=jax.ShapeDtypeStruct((S, D), A_x.dtype),
        in_specs=[hbm, vmem, hbm, hbm, hbm, hbm, hbm, hbm, vmem],
        out_specs=hbm,
        scratch_shapes=[
            pltpu.VMEM((S, D), BF16),
            pltpu.VMEM((D, 3 * D), BF16),
            pltpu.VMEM((D, D), BF16),
            pltpu.VMEM((3 * D, LANES), F32),
            pltpu.VMEM((nc, 3 * D, LANES), BF16),
            pltpu.VMEM((nc, D, LANES), BF16),
            pltpu.VMEM((3, (H + 4) * dh, D), BF16),
            pltpu.VMEM((3 * H * dh // LANES, D // 2, LANES), jnp.uint32),
            pltpu.VMEM((H * dh, D), BF16),
            *[pltpu.VMEM((B_ROWS, D), F32),
              pltpu.VMEM((nc, B_HALO + B_ROWS, LANES), F32),
              pltpu.VMEM((nc, B_HALO + B_ROWS, LANES), F32),
              pltpu.VMEM((B_ROWS, D), BF16)] * 2,
            pltpu.VMEM((S, D), F32),
            pltpu.VMEM((S, D), A_x.dtype),
            pltpu.SemaphoreType.DMA((2,)),
            pltpu.SemaphoreType.DMA((nc + 1,)),
            pltpu.SemaphoreType.DMA((4, S // (2 * B_ROWS))),
            pltpu.SemaphoreType.DMA(()),
        ],
        compiler_params=pltpu.CompilerParams(vmem_limit_bytes=112 * 2**20),
    )(A_x.reshape(S, D), A_mem0.reshape(M, D), wt(A_Wq), wt(A_Wk), wt(A_Wv),
      A_Wo.reshape(H * dh, D), B_wqkv, B_wo, gate_w.reshape(1, D))
    return out.reshape(B, S, D)
```

```python
import functools

import jax
import jax.numpy as jnp
import jax.experimental.pallas as pl
import jax.experimental.pallas.tpu as pltpu

F32 = jnp.float32
BF16 = jnp.bfloat16
NEG = -1000000000.0
LANES = 128

B_HEADS, B_WIN, B_DIL = 32, 8, 2
B_HALO = 16
B_ROWS = 128
B_SUB = 32
V_LAG, O_LAG = 3, 4
A_UNROLL = 3


def _dot(a, b):
    return jax.lax.dot_general(a, b, (((1,), (0,)), ((), ())), preferred_element_type=F32)


def _dot_nt(a, b):
    return jax.lax.dot_general(a, b, (((1,), (1,)), ((), ())), preferred_element_type=F32)


def _iota(shape, dim):
    return jax.lax.broadcasted_iota(jnp.int32, shape, dim)


def _tile(c):
    return slice(c * LANES, (c + 1) * LANES)


def _dot_tiles(a, w_ref, first, n):
    w = jnp.concatenate([w_ref[first + c] for c in range(n)], axis=1)
    return _dot(a, pltpu.bitcast(w, BF16))


def _interleave(*gens):
    gens = list(gens)
    while gens:
        gens = [g for g in gens if next(g, StopIteration) is not StopIteration]


def _gate(x, gw):
    return jax.nn.sigmoid(jnp.sum(x * gw, axis=-1, keepdims=True))


def _kernel(x_hbm, mem0_ref, wq_hbm, wk_hbm, wv_hbm, wo_hbm, bqkv_hbm, bo_hbm, gw_ref,
            out_hbm,
            x_v, bqkv_v, bo_v, tmp_s, bqkv_p, bo_p, stage, w_all, wo_v, bq0, bk0, bv0, ba0, bq1, bk1, bv1, ba1, gb_s,
            out_v, sem_o, sem_b, sem_w, sem_out, *, seg, dh):
    S, D = x_v.shape
    M = mem0_ref.shape[0]
    L = M + seg
    n_seg = S // seg
    PW = 2 * dh
    n_pair = wo_v.shape[0] // PW
    n_blk = S // (2 * B_ROWS)
    ppb = n_pair // n_blk
    nc = D // LANES
    ntp = PW // LANES
    assert ppb == 2
    bdh = D // B_HEADS

    def cp_bqkv(i):
        rows = pl.ds(i * LANES, LANES)
        return pltpu.make_async_copy(bqkv_hbm.at[rows], bqkv_v.at[rows], sem_b.at[i])

    cp_bo = pltpu.make_async_copy(bo_hbm, bo_v, sem_b.at[nc])

    def cp_x(i):
        rows = pl.ds(i * (2 * B_ROWS), 2 * B_ROWS)
        return pltpu.make_async_copy(x_hbm.at[rows], x_v.at[rows], sem_w.at[3, i])

    def cp_w(j, i):
        n = ppb * PW
        return pltpu.make_async_copy((wq_hbm, wk_hbm, wv_hbm)[j].at[pl.ds(i * n, n)],
                                     stage.at[j, pl.ds((i + 1) * n, n)], sem_w.at[j, i])

    def cp_wo(i):
        rows = pl.ds(i * (n_pair * dh), n_pair * dh)
        return pltpu.make_async_copy(wo_hbm.at[rows], wo_v.at[rows], sem_o.at[i])

    def reorder_rows(dst, c, row0):
        for d in range(bdh):
            t = tmp_s[pl.ds(row0 + d, B_HEADS, stride=bdh), :]
            rows = pl.ds((row0 + d * B_HEADS) // 2, B_HEADS // 2)
            dst[c, rows, :] = pltpu.bitcast(t.astype(BF16), jnp.uint32)

    buf0, buf1 = (bq0, bk0, bv0, ba0), (bq1, bk1, bv1, ba1)
    cp_bqkv(0).start()
    cp_bqkv(1).start()
    for ref in (bq1, bk1, bv1):
        ref[...] = jnp.zeros(ref.shape, ref.dtype)
    stage[:, :ppb * PW, :] = jnp.zeros((3, ppb * PW, D), BF16)
    for i in range(nc):
        cp_bqkv(i).wait()
        if i + 2 < nc:
            cp_bqkv(i + 2).start()
        if i == 3:
            cp_x(0).start()
            cp_bo.start()
        if i == 4:
            cp_x(1).start()
            for j in range(3):
                cp_w(j, 0).start()
        for j in range(3):
            tmp_s[j * D:(j + 1) * D, :] = bqkv_v[_tile(i), j * D:(j + 1) * D].astype(F32).T
            reorder_rows(bqkv_p, i, j * D)
    cp_bo.wait()
    for cc in range(nc):
        tmp_s[0:D, :] = bo_v[:, _tile(cc)].astype(F32)
        reorder_rows(bo_p, cc, 0)

    gw = gw_ref[...].astype(F32).reshape(1, D)

    def b_proj(r0, buf, prev, first):
        q_s, k_s, v_s, _ = buf
        xb = x_v[pl.ds(r0, B_ROWS), :]

        def proj(t):
            w = jnp.concatenate(
                [bqkv_p[c, t * (D // 2):(t + 1) * (D // 2), :] for c in range(nc)], axis=1)
            return _dot_nt(xb, pltpu.bitcast(w, BF16))

        for t, dst, src in ((1, k_s, prev[1]), (2, v_s, prev[2])):
            y = proj(t)
            for cc in range(nc):
                yc = y[:, _tile(cc)]
                halo = src[cc, B_ROWS:, :]
                if first is not None:
                    halo = jnp.where(first, jnp.broadcast_to(yc[0:1], halo.shape), halo)
                dst[cc, :B_HALO, :] = halo
                dst[cc, B_HALO:, :] = yc
            yield
        q_s[...] = proj(0) * (bdh ** -0.5)
        yield

    def w_transpose(p):
        rows = pl.ds(pl.multiple_of((p + ppb) * PW, PW), PW)
        for j in range(3):
            t = stage[j, rows, :].T
            for c in range(ntp):
                w_all[(jnp.maximum(p, 0) * 3 + j) * ntp + c] = pltpu.bitcast(t[:, _tile(c)], jnp.uint32)
            yield

    def b_attn(r0, buf, first):
        q_s, k_s, v_s, att_s = buf
        half = B_WIN // 2
        shift = half * B_DIL
        for sb in range(B_ROWS // B_SUB):
            base = B_HALO + sb * B_SUB
            out_rows = slice(sb * B_SUB, (sb + 1) * B_SUB)
            logits = [None] * B_WIN
            for cc in range(nc):
                q = q_s[out_rows, _tile(cc)]
                for w in range(half):
                    k = k_s[cc, pl.ds(base - w * B_DIL - shift, B_SUB + shift), :]
                    for ww, kk in ((w, k[shift:]), (w + half, k[:B_SUB])):
                        logits[ww] = q * kk if cc == 0 else logits[ww] + q * kk
            for w in range(B_WIN):
                t = logits[w]
                t = t + pltpu.roll(t, 2 * B_HEADS, 1)
                t = t + pltpu.roll(t, B_HEADS, 1)
                if first is not None and sb * B_SUB < w * B_DIL:
                    pos = r0 + sb * B_SUB + _iota((B_SUB, LANES), 0)
                    t = jnp.where(pos >= w * B_DIL, t, NEG)
                logits[w] = t
            mx = functools.reduce(jnp.maximum, logits)
            e = [jnp.exp(t - mx) for t in logits]
            inv = 1.0 / functools.reduce(jnp.add, e)
            for cc in range(nc):
                o = None
                for w in range(half):
                    v = v_s[cc, pl.ds(base - w * B_DIL - shift, B_SUB + shift), :]
                    t = e[w] * v[shift:] + e[w + half] * v[:B_SUB]
                    o = t if o is None else o + t
                att_s[out_rows, _tile(cc)] = (o * inv).astype(BF16)
            yield

    def b_out(r0, buf):
        rows = pl.ds(r0, B_ROWS)
        b = _dot_tiles(buf[3][...], bo_p, 0, nc)
        gb_s[rows, :] = (1.0 - _gate(x_v[rows, :].astype(F32), gw)) * b

    def b_block(i, _):
        @pl.when(i + 2 < n_blk)
        def _():
            cp_x(i + 2).start()

        @pl.when(i + 1 < n_blk)
        def _():
            for j in range(3):
                cp_w(j, i + 1).start()

        @pl.when(i + 2 >= n_blk)
        def _():
            cp_wo(i + 2 - n_blk).start()

        @pl.when(i > 0)
        def _():
            for j in range(3):
                cp_w(j, i - 1).wait()

        cp_x(i).wait()
        r0 = pl.multiple_of(i * (2 * B_ROWS), B_ROWS)
        r1 = pl.multiple_of(r0 + B_ROWS, B_ROWS)
        r_prev = pl.multiple_of(jnp.maximum(r0 - B_ROWS, 0), B_ROWS)
        _interleave(b_proj(r0, buf0, buf1, i == 0), b_attn(r_prev, buf1, None),
                    w_transpose((i - 1) * ppb))
        b_out(r_prev, buf1)
        _interleave(b_proj(r1, buf1, buf0, None), b_attn(r0, buf0, i == 0),
                    w_transpose((i - 1) * ppb + 1))
        b_out(r0, buf0)
        return None

    jax.lax.fori_loop(0, n_blk, b_block, None)

    def b_tail():
        yield from b_attn(S - B_ROWS, buf1, None)
        b_out(S - B_ROWS, buf1)
        for j in range(3):
            cp_w(j, n_blk - 1).wait()
        for p in range(n_pair - ppb, n_pair):
            yield from w_transpose(p)

    row, lane = _iota((L, 2 * L), 0), _iota((L, 2 * L), 1)
    is_a = lane < L
    key = jnp.where(is_a, lane, lane - L)
    keep = (row < M) | (row >= key)
    lo_half = _iota((L, LANES), 1) < dh - LANES
    zeros = jnp.zeros((L, LANES), F32)
    scale = dh ** -0.5

    def split_heads(t):
        mid = t[:, LANES:2 * LANES]
        top = jnp.concatenate([t[:, :LANES], jnp.where(lo_half, mid, 0.0), zeros], axis=1)
        bot = jnp.concatenate([zeros, jnp.where(lo_half, 0.0, mid), t[:, 2 * LANES:]], axis=1)
        return jnp.concatenate([top, bot], axis=0).astype(BF16)

    def softmax(s):
        s = jnp.where(keep, s * scale, NEG)
        m_a = jnp.max(jnp.where(is_a, s, -jnp.inf), axis=1, keepdims=True)
        m_b = jnp.max(jnp.where(is_a, -jnp.inf, s), axis=1, keepdims=True)
        e = jnp.exp(s - jnp.where(is_a, m_a, m_b))
        l_a = jnp.sum(jnp.where(is_a, e, 0.0), axis=1, keepdims=True)
        l_b = jnp.sum(jnp.where(is_a, 0.0, e), axis=1, keepdims=True)
        return e / jnp.where(is_a, l_a, l_b)

    def a_step(s, mem, o_lag=O_LAG, side=iter(()), before_out=lambda: None):
        rows = pl.ds(pl.multiple_of(s * seg, seg), seg)
        xs = x_v[rows, :].astype(F32)
        h = jnp.concatenate([mem, xs], axis=0)
        q, kb, vb, prob, att = {}, {}, {}, {}, {}
        acc = None
        for t in range(n_pair + V_LAG + 1):
            next(side, None)
            if t < n_pair:
                q[t] = _dot_tiles(h, w_all, 3 * t * ntp, ntp)
                kb[t] = split_heads(_dot_tiles(h, w_all, (3 * t + 1) * ntp, ntp))
            p = t - V_LAG
            if 0 <= p < n_pair:
                vb[p] = split_heads(_dot_tiles(h, w_all, (3 * p + 2) * ntp, ntp))
            p = t - 1
            if 0 <= p < n_pair:
                prob[p] = softmax(_dot_nt(q.pop(p), kb.pop(p)))
            p = t - V_LAG - 1 - o_lag
            if p >= 0:
                y = _dot(att.pop(p), wo_v[p * PW:(p + 1) * PW, :])
                acc = y if acc is None else acc + y
            p = t - V_LAG - 1
            if p >= 0:
                att[p] = _dot(prob.pop(p), vb.pop(p))
        before_out()
        rest = jnp.concatenate([att[p] for p in sorted(att)], axis=1)
        o = jnp.concatenate(
            [_dot(rest, wo_v[(n_pair - o_lag) * PW:, _tile(c)]) for c in range(nc)], axis=1)
        o = o if acc is None else acc + o
        out_v[rows, :] = (_gate(xs, gw) * o[M:] + gb_s[rows, :]).astype(out_v.dtype)
        return o[:M].astype(BF16).astype(F32)

    def store_out(s, n):
        rows = pl.ds(pl.multiple_of(s * seg, seg), n * seg)
        pltpu.make_async_copy(out_v.at[rows], out_hbm.at[rows], sem_out).start()

    def a_group(g, mem):
        s0 = 1 + g * A_UNROLL
        for u in range(A_UNROLL):
            mem = a_step(s0 + u, mem)
        store_out(s0, A_UNROLL)
        return mem

    def wait_wo():
        cp_wo(0).wait()
        cp_wo(1).wait()

    mem = a_step(0, mem0_ref[...].astype(F32), n_pair, b_tail(), wait_wo)
    store_out(0, 1)
    assert (n_seg - 1) % A_UNROLL == 0
    jax.lax.fori_loop(0, (n_seg - 1) // A_UNROLL, a_group, mem)
    pltpu.make_async_copy(out_v, out_hbm, sem_out).wait()


@functools.partial(jax.jit, static_argnames=("A_seg_len",))
def pallas_gated_mix__memory_aug_recurrent_mem_tr__sliding_local_dilated__prompt_kernel(
    A_x, A_mem0, A_Wq, A_Wk, A_Wv, A_Wo, A_seg_len, B_x, B_wqkv, B_wo, gate_w,
):
    del B_x
    B, S, D = A_x.shape
    M = A_mem0.shape[1]
    H, dh = A_Wq.shape[1:]
    seg = int(A_seg_len)
    L = M + seg
    assert B == 1 and S % (2 * B_ROWS) == 0 and S % seg == 0 and 2 * dh == 3 * LANES and 2 * L <= LANES
    nc = D // LANES

    def wt(w):
        return w.transpose(1, 2, 0).reshape(H * dh, D)

    hbm = pl.BlockSpec(memory_space=pl.ANY)
    vmem = pl.BlockSpec(memory_space=pltpu.VMEM)
    out = pl.pallas_call(
        functools.partial(_kernel, seg=seg, dh=dh),
        out_shape=jax.ShapeDtypeStruct((S, D), A_x.dtype),
        in_specs=[hbm, vmem, hbm, hbm, hbm, hbm, hbm, hbm, vmem],
        out_specs=hbm,
        scratch_shapes=[
            pltpu.VMEM((S, D), BF16),
            pltpu.VMEM((D, 3 * D), BF16),
            pltpu.VMEM((D, D), BF16),
            pltpu.VMEM((3 * D, LANES), F32),
            pltpu.VMEM((nc, 3 * D // 2, LANES), jnp.uint32),
            pltpu.VMEM((nc, D // 2, LANES), jnp.uint32),
            pltpu.VMEM((3, (H + 4) * dh, D), BF16),
            pltpu.VMEM((3 * H * dh // LANES, D // 2, LANES), jnp.uint32),
            pltpu.VMEM((H * dh, D), BF16),
            *[pltpu.VMEM((B_ROWS, D), F32),
              pltpu.VMEM((nc, B_HALO + B_ROWS, LANES), F32),
              pltpu.VMEM((nc, B_HALO + B_ROWS, LANES), F32),
              pltpu.VMEM((B_ROWS, D), BF16)] * 2,
            pltpu.VMEM((S, D), F32),
            pltpu.VMEM((S, D), A_x.dtype),
            pltpu.SemaphoreType.DMA((2,)),
            pltpu.SemaphoreType.DMA((nc + 1,)),
            pltpu.SemaphoreType.DMA((4, S // (2 * B_ROWS))),
            pltpu.SemaphoreType.DMA(()),
        ],
        compiler_params=pltpu.CompilerParams(vmem_limit_bytes=112 * 2**20),
    )(A_x.reshape(S, D), A_mem0.reshape(M, D), wt(A_Wq), wt(A_Wk), wt(A_Wv),
      A_Wo.reshape(H * dh, D), B_wqkv, B_wo, gate_w)
    return out.reshape(B, S, D)
```

```python
import functools

import jax
import jax.numpy as jnp
import jax.experimental.pallas as pl
import jax.experimental.pallas.tpu as pltpu

F32 = jnp.float32
BF16 = jnp.bfloat16
NEG = -1000000000.0
LANES = 128

B_HEADS, B_WIN, B_DIL = 32, 8, 2
B_HALO = 16
B_ROWS = 128
B_SUB = 32
V_LAG, O_LAG = 3, 4
A_UNROLL = 3


def _dot(a, b):
    return jax.lax.dot_general(a, b, (((1,), (0,)), ((), ())), preferred_element_type=F32)


def _dot_nt(a, b):
    return jax.lax.dot_general(a, b, (((1,), (1,)), ((), ())), preferred_element_type=F32)


def _iota(shape, dim):
    return jax.lax.broadcasted_iota(jnp.int32, shape, dim)


def _tile(c):
    return slice(c * LANES, (c + 1) * LANES)


def _dot_tiles(a, w_ref, first, n):
    w = jnp.concatenate([w_ref[first + c] for c in range(n)], axis=1)
    return _dot(a, pltpu.bitcast(w, BF16))


def _interleave(*gens):
    gens = list(gens)
    while gens:
        gens = [g for g in gens if next(g, StopIteration) is not StopIteration]


def _gate(x, gw):
    return jax.nn.sigmoid(jnp.sum(x * gw, axis=-1, keepdims=True))


def _kernel(x_hbm, mem0_ref, wq_hbm, wk_hbm, wv_hbm, wo_hbm, bqkv_hbm, bo_hbm, gw_ref,
            out_hbm,
            x_v, bqkv_v, bo_v, tmp_s, bqkv_p, bo_p, stage, w_all, wo_v,
            bq0, bk0, bv0, ba0, bq1, bk1, bv1, ba1, gb_s,
            out_v, sem_o, sem_b, sem_w, sem_out, *, seg, dh):
    S, D = x_v.shape
    M = mem0_ref.shape[0]
    L = M + seg
    n_seg = S // seg
    PW = 2 * dh
    n_pair = wo_v.shape[0] // PW
    n_blk = S // (2 * B_ROWS)
    ppb = n_pair // n_blk
    nc = D // LANES
    ntp = PW // LANES
    bdh = D // B_HEADS
    assert ppb == 2 and LANES == 4 * B_HEADS

    def cp_bqkv(i):
        rows = pl.ds(i * LANES, LANES)
        return pltpu.make_async_copy(bqkv_hbm.at[rows], bqkv_v.at[rows], sem_b.at[i])

    cp_bo = pltpu.make_async_copy(bo_hbm, bo_v, sem_b.at[nc])

    def cp_x(i):
        rows = pl.ds(i * (2 * B_ROWS), 2 * B_ROWS)
        return pltpu.make_async_copy(x_hbm.at[rows], x_v.at[rows], sem_w.at[3, i])

    def cp_w(j, i):
        n = ppb * PW
        return pltpu.make_async_copy((wq_hbm, wk_hbm, wv_hbm)[j].at[pl.ds(i * n, n)],
                                     stage.at[j, pl.ds((i + 1) * n, n)], sem_w.at[j, i])

    def cp_wo(i):
        rows = pl.ds(i * (n_pair * dh), n_pair * dh)
        return pltpu.make_async_copy(wo_hbm.at[rows], wo_v.at[rows], sem_o.at[i])

    def reorder_rows(dst, c, row0):
        for d in range(bdh):
            t = tmp_s[pl.ds(row0 + d, B_HEADS, stride=bdh), :]
            rows = pl.ds((row0 + d * B_HEADS) // 2, B_HEADS // 2)
            dst[c, rows, :] = pltpu.bitcast(t.astype(BF16), jnp.uint32)

    buf0, buf1 = (bq0, bk0, bv0, ba0), (bq1, bk1, bv1, ba1)
    cp_bqkv(0).start()
    cp_bqkv(1).start()
    for ref in (bq1, bk1, bv1):
        ref[...] = jnp.zeros(ref.shape, ref.dtype)
    stage[:, :ppb * PW, :] = jnp.zeros((3, ppb * PW, D), BF16)
    for i in range(nc):
        cp_bqkv(i).wait()
        if i + 2 < nc:
            cp_bqkv(i + 2).start()
        if i == 3:
            cp_x(0).start()
            cp_bo.start()
        if i == 4:
            cp_x(1).start()
            for j in range(3):
                cp_w(j, 0).start()
        for j in range(3):
            tmp_s[j * D:(j + 1) * D, :] = bqkv_v[_tile(i), j * D:(j + 1) * D].astype(F32).T
            reorder_rows(bqkv_p, i, j * D)
    cp_bo.wait()
    for cc in range(nc):
        tmp_s[0:D, :] = bo_v[:, _tile(cc)].astype(F32)
        reorder_rows(bo_p, cc, 0)

    gw = gw_ref[...].astype(F32).reshape(1, D)

    def b_proj(r0, buf, prev, first):
        q_s, k_s, v_s, _ = buf
        xb = x_v[pl.ds(r0, B_ROWS), :]

        def proj(t):
            w = jnp.concatenate(
                [bqkv_p[c, t * (D // 2):(t + 1) * (D // 2), :] for c in range(nc)], axis=1)
            return _dot_nt(xb, pltpu.bitcast(w, BF16))

        for t, dst, src in ((1, k_s, prev[1]), (2, v_s, prev[2])):
            y = proj(t)
            for cc in range(nc):
                yc = y[:, _tile(cc)]
                halo = src[cc, B_ROWS:, :]
                if first is not None:
                    halo = jnp.where(first, jnp.broadcast_to(yc[0:1], halo.shape), halo)
                dst[cc, :B_HALO, :] = halo
                dst[cc, B_HALO:, :] = yc
            yield
        q_s[...] = proj(0) * (bdh ** -0.5)
        yield

    def w_transpose(p):
        rows = pl.ds(pl.multiple_of((p + ppb) * PW, PW), PW)
        for j in range(3):
            t = stage[j, rows, :].T
            for c in range(ntp):
                w_all[(jnp.maximum(p, 0) * 3 + j) * ntp + c] = pltpu.bitcast(t[:, _tile(c)], jnp.uint32)
            yield

    def b_attn(r0, buf, first):
        q_s, k_s, v_s, att_s = buf
        half = B_WIN // 2
        shift = half * B_DIL
        for sb in range(B_ROWS // B_SUB):
            base = B_HALO + sb * B_SUB
            out_rows = slice(sb * B_SUB, (sb + 1) * B_SUB)
            logits = [None] * B_WIN
            for cc in range(nc):
                q = q_s[out_rows, _tile(cc)]
                for w in range(half):
                    k = k_s[cc, pl.ds(base - w * B_DIL - shift, B_SUB + shift), :]
                    for ww, kk in ((w, k[shift:]), (w + half, k[:B_SUB])):
                        logits[ww] = q * kk if cc == 0 else logits[ww] + q * kk
            for w in range(B_WIN):
                t = logits[w]
                t = t + pltpu.roll(t, 2 * B_HEADS, 1)
                t = t + pltpu.roll(t, B_HEADS, 1)
                if first is not None and sb * B_SUB < w * B_DIL:
                    pos = r0 + sb * B_SUB + _iota((B_SUB, LANES), 0)
                    t = jnp.where(pos >= w * B_DIL, t, NEG)
                logits[w] = t
            mx = functools.reduce(jnp.maximum, logits)
            e = [jnp.exp(t - mx) for t in logits]
            inv = 1.0 / functools.reduce(jnp.add, e)
            for cc in range(nc):
                o = None
                for w in range(half):
                    v = v_s[cc, pl.ds(base - w * B_DIL - shift, B_SUB + shift), :]
                    t = e[w] * v[shift:] + e[w + half] * v[:B_SUB]
                    o = t if o is None else o + t
                att_s[out_rows, _tile(cc)] = (o * inv).astype(BF16)
            yield

    def b_out(r0, buf):
        rows = pl.ds(r0, B_ROWS)
        b = _dot_tiles(buf[3][...], bo_p, 0, nc)
        gb_s[rows, :] = (1.0 - _gate(x_v[rows, :].astype(F32), gw)) * b

    def b_block(i, _):
        @pl.when(i + 2 < n_blk)
        def _():
            cp_x(i + 2).start()

        @pl.when(i + 1 < n_blk)
        def _():
            for j in range(3):
                cp_w(j, i + 1).start()

        @pl.when(i + 2 >= n_blk)
        def _():
            cp_wo(i + 2 - n_blk).start()

        @pl.when(i > 0)
        def _():
            for j in range(3):
                cp_w(j, i - 1).wait()

        cp_x(i).wait()
        r0 = pl.multiple_of(i * (2 * B_ROWS), B_ROWS)
        r1 = pl.multiple_of(r0 + B_ROWS, B_ROWS)
        r_prev = pl.multiple_of(jnp.maximum(r0 - B_ROWS, 0), B_ROWS)
        _interleave(b_proj(r0, buf0, buf1, i == 0), b_attn(r_prev, buf1, None),
                    w_transpose((i - 1) * ppb))
        b_out(r_prev, buf1)
        _interleave(b_proj(r1, buf1, buf0, None), b_attn(r0, buf0, i == 0),
                    w_transpose((i - 1) * ppb + 1))
        b_out(r0, buf0)
        return None

    jax.lax.fori_loop(0, n_blk, b_block, None)

    def b_tail():
        yield from b_attn(S - B_ROWS, buf1, None)
        b_out(S - B_ROWS, buf1)
        for j in range(3):
            cp_w(j, n_blk - 1).wait()
        for p in range(n_pair - ppb, n_pair):
            yield from w_transpose(p)

    row, lane = _iota((L, 2 * L), 0), _iota((L, 2 * L), 1)
    is_a = lane < L
    key = jnp.where(is_a, lane, lane - L)
    keep = (row < M) | (row >= key)
    lo_half = _iota((L, LANES), 1) < dh - LANES
    zeros = jnp.zeros((L, LANES), F32)
    scale = dh ** -0.5

    def split_heads(t):
        mid = t[:, LANES:2 * LANES]
        top = jnp.concatenate([t[:, :LANES], jnp.where(lo_half, mid, 0.0), zeros], axis=1)
        bot = jnp.concatenate([zeros, jnp.where(lo_half, 0.0, mid), t[:, 2 * LANES:]], axis=1)
        return jnp.concatenate([top, bot], axis=0).astype(BF16)

    def softmax(s):
        s = jnp.where(keep, s * scale, NEG)
        m_a = jnp.max(jnp.where(is_a, s, -jnp.inf), axis=1, keepdims=True)
        m_b = jnp.max(jnp.where(is_a, -jnp.inf, s), axis=1, keepdims=True)
        e = jnp.exp(s - jnp.where(is_a, m_a, m_b))
        l_a = jnp.sum(jnp.where(is_a, e, 0.0), axis=1, keepdims=True)
        l_b = jnp.sum(jnp.where(is_a, 0.0, e), axis=1, keepdims=True)
        return e / jnp.where(is_a, l_a, l_b)

    def a_step(s, mem, o_lag=O_LAG, side=iter(()), before_out=lambda: None):
        rows = pl.ds(pl.multiple_of(s * seg, seg), seg)
        xs = x_v[rows, :].astype(F32)
        h = jnp.concatenate([xs, mem], axis=0)

        def proj(j, p):
            y = _dot_tiles(h, w_all, (3 * p + j) * ntp, ntp)
            return jnp.concatenate([y[seg:], y[:seg]], axis=0)

        q, kb, vb, prob, att = {}, {}, {}, {}, {}
        acc = None
        for t in range(n_pair + V_LAG + 1):
            next(side, None)
            if t < n_pair:
                q[t] = proj(0, t)
                kb[t] = split_heads(proj(1, t))
            p = t - V_LAG
            if 0 <= p < n_pair:
                vb[p] = split_heads(proj(2, p))
            p = t - 1
            if 0 <= p < n_pair:
                prob[p] = softmax(_dot_nt(q.pop(p), kb.pop(p)))
            p = t - V_LAG - 1 - o_lag
            if p >= 0:
                y = _dot(att.pop(p), wo_v[p * PW:(p + 1) * PW, :])
                acc = y if acc is None else acc + y
            p = t - V_LAG - 1
            if p >= 0:
                att[p] = _dot(prob.pop(p), vb.pop(p))
        before_out()
        rest = jnp.concatenate([att[p] for p in sorted(att)], axis=1)
        o = jnp.concatenate(
            [_dot(rest, wo_v[(n_pair - o_lag) * PW:, _tile(c)]) for c in range(nc)], axis=1)
        o = o if acc is None else acc + o
        out_v[rows, :] = (_gate(xs, gw) * o[M:] + gb_s[rows, :]).astype(out_v.dtype)
        return o[:M].astype(BF16).astype(F32)

    def store_out(s, n):
        rows = pl.ds(pl.multiple_of(s * seg, seg), n * seg)
        pltpu.make_async_copy(out_v.at[rows], out_hbm.at[rows], sem_out).start()

    def a_group(g, mem):
        s0 = 1 + g * A_UNROLL
        for u in range(A_UNROLL):
            mem = a_step(s0 + u, mem)
        store_out(s0, A_UNROLL)
        return mem

    def wait_wo():
        cp_wo(0).wait()
        cp_wo(1).wait()

    mem = a_step(0, mem0_ref[...].astype(F32), n_pair, b_tail(), wait_wo)
    store_out(0, 1)
    assert (n_seg - 1) % A_UNROLL == 0
    jax.lax.fori_loop(0, (n_seg - 1) // A_UNROLL, a_group, mem)
    pltpu.make_async_copy(out_v, out_hbm, sem_out).wait()


@functools.partial(jax.jit, static_argnames=("A_seg_len",))
def pallas_gated_mix__memory_aug_recurrent_mem_tr__sliding_local_dilated__prompt_kernel(
    A_x, A_mem0, A_Wq, A_Wk, A_Wv, A_Wo, A_seg_len, B_x, B_wqkv, B_wo, gate_w,
):
    del B_x
    B, S, D = A_x.shape
    M = A_mem0.shape[1]
    H, dh = A_Wq.shape[1:]
    seg = int(A_seg_len)
    L = M + seg
    assert B == 1 and S % (2 * B_ROWS) == 0 and S % seg == 0 and 2 * dh == 3 * LANES and 2 * L <= LANES
    nc = D // LANES

    def wt(w):
        return w.transpose(1, 2, 0).reshape(H * dh, D)

    hbm = pl.BlockSpec(memory_space=pl.ANY)
    vmem = pl.BlockSpec(memory_space=pltpu.VMEM)
    out = pl.pallas_call(
        functools.partial(_kernel, seg=seg, dh=dh),
        out_shape=jax.ShapeDtypeStruct((S, D), A_x.dtype),
        in_specs=[hbm, vmem, hbm, hbm, hbm, hbm, hbm, hbm, vmem],
        out_specs=hbm,
        scratch_shapes=[
            pltpu.VMEM((S, D), BF16),
            pltpu.VMEM((D, 3 * D), BF16),
            pltpu.VMEM((D, D), BF16),
            pltpu.VMEM((3 * D + B_HEADS, LANES), F32),
            pltpu.VMEM((nc, 3 * D // 2, LANES), jnp.uint32),
            pltpu.VMEM((nc, D // 2, LANES), jnp.uint32),
            pltpu.VMEM((3, (H + 4) * dh, D), BF16),
            pltpu.VMEM((3 * H * dh // LANES, D // 2, LANES), jnp.uint32),
            pltpu.VMEM((H * dh, D), BF16),
            *[pltpu.VMEM((B_ROWS, D), F32),
              pltpu.VMEM((nc, B_HALO + B_ROWS, LANES), F32),
              pltpu.VMEM((nc, B_HALO + B_ROWS, LANES), F32),
              pltpu.VMEM((B_ROWS, D), BF16)] * 2,
            pltpu.VMEM((S, D), F32),
            pltpu.VMEM((S, D), A_x.dtype),
            pltpu.SemaphoreType.DMA((2,)),
            pltpu.SemaphoreType.DMA((nc + 1,)),
            pltpu.SemaphoreType.DMA((4, S // (2 * B_ROWS))),
            pltpu.SemaphoreType.DMA(()),
        ],
        compiler_params=pltpu.CompilerParams(vmem_limit_bytes=112 * 2**20),
    )(A_x.reshape(S, D), A_mem0.reshape(M, D), wt(A_Wq), wt(A_Wk), wt(A_Wv),
      A_Wo.reshape(H * dh, D), B_wqkv, B_wo, gate_w)
    return out.reshape(B, S, D)
```

```python
import functools

import jax
import jax.numpy as jnp
import jax.experimental.pallas as pl
import jax.experimental.pallas.tpu as pltpu

F32 = jnp.float32
BF16 = jnp.bfloat16
NEG = -1000000000.0
LANES = 128

B_HEADS, B_WIN, B_DIL = 32, 8, 2
B_HALO = 16
B_ROWS = 128
B_SUB = 32
V_LAG, O_LAG = 3, 4
A_UNROLL = 3


def _dot(a, b):
    return jax.lax.dot_general(a, b, (((1,), (0,)), ((), ())), preferred_element_type=F32)


def _dot_nt(a, b):
    return jax.lax.dot_general(a, b, (((1,), (1,)), ((), ())), preferred_element_type=F32)


def _iota(shape, dim):
    return jax.lax.broadcasted_iota(jnp.int32, shape, dim)


def _tile(c):
    return slice(c * LANES, (c + 1) * LANES)


def _dot_tiles(a, w_ref, first, n):
    w = jnp.concatenate([w_ref[first + c] for c in range(n)], axis=1)
    return _dot(a, pltpu.bitcast(w, BF16))


def _interleave(*gens):
    gens = list(gens)
    while gens:
        gens = [g for g in gens if next(g, StopIteration) is not StopIteration]


def _gate(x, gw):
    return jax.nn.sigmoid(jnp.sum(x * gw, axis=-1, keepdims=True))


def _kernel(x_hbm, mem0_ref, wq_hbm, wk_hbm, wv_hbm, wo_hbm, bqkv_hbm, bo_hbm, gw_ref,
            out_hbm,
            x_v, bqkv_v, bo_v, tmp_s, bqkv_p, bo_p, stage, w_all, wo_v,
            bq0, bk0, bv0, ba0, bq1, bk1, bv1, ba1, gb_s,
            out_v, sem_o, sem_b, sem_w, sem_out, *, seg, dh):
    S, D = x_v.shape
    M = mem0_ref.shape[0]
    L = M + seg
    n_seg = S // seg
    PW = 2 * dh
    n_pair = wo_v.shape[0] // PW
    n_blk = S // (2 * B_ROWS)
    ppb = n_pair // n_blk
    nc = D // LANES
    ntp = PW // LANES
    bdh = D // B_HEADS
    assert ppb == 2 and LANES == 4 * B_HEADS

    def cp_bqkv(i):
        rows = pl.ds(i * LANES, LANES)
        return pltpu.make_async_copy(bqkv_hbm.at[rows], bqkv_v.at[rows], sem_b.at[i])

    cp_bo = pltpu.make_async_copy(bo_hbm, bo_v, sem_b.at[nc])

    def cp_x(i):
        rows = pl.ds(i * (2 * B_ROWS), 2 * B_ROWS)
        return pltpu.make_async_copy(x_hbm.at[rows], x_v.at[rows], sem_w.at[3, i])

    def cp_w(j, i):
        n = ppb * PW
        return pltpu.make_async_copy((wq_hbm, wk_hbm, wv_hbm)[j].at[pl.ds(i * n, n)],
                                     stage.at[j, pl.ds((i + 1) * n, n)], sem_w.at[j, i])

    def cp_wo(i):
        rows = pl.ds(i * (n_pair * dh), n_pair * dh)
        return pltpu.make_async_copy(wo_hbm.at[rows], wo_v.at[rows], sem_o.at[i])

    def reorder_rows(dst, c, row0):
        for d in range(bdh):
            t = tmp_s[pl.ds(row0 + d, B_HEADS, stride=bdh), :]
            rows = pl.ds((row0 + d * B_HEADS) // 2, B_HEADS // 2)
            dst[c, rows, :] = pltpu.bitcast(t.astype(BF16), jnp.uint32)

    buf0, buf1 = (bq0, bk0, bv0, ba0), (bq1, bk1, bv1, ba1)
    cp_bo.start()
    cp_bqkv(0).start()
    for ref in (bq1, bk1, bv1):
        ref[...] = jnp.zeros(ref.shape, ref.dtype)
    stage[:, :ppb * PW, :] = jnp.zeros((3, ppb * PW, D), BF16)
    cp_bo.wait()
    cp_bqkv(1).start()
    for cc in range(nc):
        tmp_s[0:D, :] = bo_v[:, _tile(cc)].astype(F32)
        reorder_rows(bo_p, cc, 0)
    for i in range(nc):
        cp_bqkv(i).wait()
        if i + 2 < nc:
            cp_bqkv(i + 2).start()
        if i == 2:
            cp_x(0).start()
        for j in range(3):
            if i == (3, 4, 4)[j]:
                cp_w(j, 0).start()
        if i == 4:
            cp_x(1).start()
        for j in range(3):
            tmp_s[j * D:(j + 1) * D, :] = bqkv_v[_tile(i), j * D:(j + 1) * D].astype(F32).T
            reorder_rows(bqkv_p, i, j * D)

    gw = gw_ref[...].astype(F32).reshape(1, D)

    def b_proj(r0, buf, prev, first):
        q_s, k_s, v_s, _ = buf
        xb = x_v[pl.ds(r0, B_ROWS), :]

        def proj(t):
            w = jnp.concatenate(
                [bqkv_p[c, t * (D // 2):(t + 1) * (D // 2), :] for c in range(nc)], axis=1)
            return _dot_nt(xb, pltpu.bitcast(w, BF16))

        for t, dst, src in ((1, k_s, prev[1]), (2, v_s, prev[2])):
            y = proj(t)
            for cc in range(nc):
                yc = y[:, _tile(cc)]
                halo = src[cc, B_ROWS:, :]
                if first is not None:
                    halo = jnp.where(first, jnp.broadcast_to(yc[0:1], halo.shape), halo)
                dst[cc, :B_HALO, :] = halo
                dst[cc, B_HALO:, :] = yc
            yield
        q_s[...] = proj(0) * (bdh ** -0.5)
        yield

    def w_transpose(p):
        rows = pl.ds(pl.multiple_of((p + ppb) * PW, PW), PW)
        for j in range(3):
            t = stage[j, rows, :].T
            for c in range(ntp):
                w_all[(jnp.maximum(p, 0) * 3 + j) * ntp + c] = pltpu.bitcast(t[:, _tile(c)], jnp.uint32)
            yield

    def b_attn(r0, buf, first):
        q_s, k_s, v_s, att_s = buf
        half = B_WIN // 2
        shift = half * B_DIL
        for sb in range(B_ROWS // B_SUB):
            base = B_HALO + sb * B_SUB
            out_rows = slice(sb * B_SUB, (sb + 1) * B_SUB)
            logits = [None] * B_WIN
            for cc in range(nc):
                q = q_s[out_rows, _tile(cc)]
                for w in range(half):
                    k = k_s[cc, pl.ds(base - w * B_DIL - shift, B_SUB + shift), :]
                    for ww, kk in ((w, k[shift:]), (w + half, k[:B_SUB])):
                        logits[ww] = q * kk if cc == 0 else logits[ww] + q * kk
            for w in range(B_WIN):
                t = logits[w]
                t = t + pltpu.roll(t, 2 * B_HEADS, 1)
                t = t + pltpu.roll(t, B_HEADS, 1)
                if first is not None and sb * B_SUB < w * B_DIL:
                    pos = r0 + sb * B_SUB + _iota((B_SUB, LANES), 0)
                    t = jnp.where(pos >= w * B_DIL, t, NEG)
                logits[w] = t
            mx = functools.reduce(jnp.maximum, logits)
            e = [jnp.exp(t - mx) for t in logits]
            inv = 1.0 / functools.reduce(jnp.add, e)
            for cc in range(nc):
                o = None
                for w in range(half):
                    v = v_s[cc, pl.ds(base - w * B_DIL - shift, B_SUB + shift), :]
                    t = e[w] * v[shift:] + e[w + half] * v[:B_SUB]
                    o = t if o is None else o + t
                att_s[out_rows, _tile(cc)] = (o * inv).astype(BF16)
            yield

    def b_out(r0, buf):
        rows = pl.ds(r0, B_ROWS)
        b = _dot_tiles(buf[3][...], bo_p, 0, nc)
        gb_s[rows, :] = (1.0 - _gate(x_v[rows, :].astype(F32), gw)) * b

    def b_block(i, _):
        @pl.when(i + 2 < n_blk)
        def _():
            cp_x(i + 2).start()

        @pl.when(i + 1 < n_blk)
        def _():
            for j in range(3):
                cp_w(j, i + 1).start()

        @pl.when(i + 2 >= n_blk)
        def _():
            cp_wo(i + 2 - n_blk).start()

        @pl.when(i > 0)
        def _():
            for j in range(3):
                cp_w(j, i - 1).wait()

        cp_x(i).wait()
        r0 = pl.multiple_of(i * (2 * B_ROWS), B_ROWS)
        r1 = pl.multiple_of(r0 + B_ROWS, B_ROWS)
        r_prev = pl.multiple_of(jnp.maximum(r0 - B_ROWS, 0), B_ROWS)
        _interleave(b_proj(r0, buf0, buf1, i == 0), b_attn(r_prev, buf1, None),
                    w_transpose((i - 1) * ppb))
        b_out(r_prev, buf1)
        _interleave(b_proj(r1, buf1, buf0, None), b_attn(r0, buf0, i == 0),
                    w_transpose((i - 1) * ppb + 1))
        b_out(r0, buf0)
        return None

    jax.lax.fori_loop(0, n_blk, b_block, None)

    def b_tail():
        yield from b_attn(S - B_ROWS, buf1, None)
        b_out(S - B_ROWS, buf1)
        for j in range(3):
            cp_w(j, n_blk - 1).wait()
        for p in range(n_pair - ppb, n_pair):
            yield from w_transpose(p)

    row, lane = _iota((L, 2 * L), 0), _iota((L, 2 * L), 1)
    is_a = lane < L
    key = jnp.where(is_a, lane, lane - L)
    keep = (row < M) | (row >= key)
    lo_half = _iota((L, LANES), 1) < dh - LANES
    zeros = jnp.zeros((L, LANES), F32)
    scale = dh ** -0.5

    def split_heads(t):
        mid = t[:, LANES:2 * LANES]
        top = jnp.concatenate([t[:, :LANES], jnp.where(lo_half, mid, 0.0), zeros], axis=1)
        bot = jnp.concatenate([zeros, jnp.where(lo_half, 0.0, mid), t[:, 2 * LANES:]], axis=1)
        return jnp.concatenate([top, bot], axis=0).astype(BF16)

    def softmax(s):
        s = jnp.where(keep, s * scale, NEG)
        m_a = jnp.max(jnp.where(is_a, s, -jnp.inf), axis=1, keepdims=True)
        m_b = jnp.max(jnp.where(is_a, -jnp.inf, s), axis=1, keepdims=True)
        e = jnp.exp(s - jnp.where(is_a, m_a, m_b))
        l_a = jnp.sum(jnp.where(is_a, e, 0.0), axis=1, keepdims=True)
        l_b = jnp.sum(jnp.where(is_a, 0.0, e), axis=1, keepdims=True)
        return e / jnp.where(is_a, l_a, l_b)

    def a_step(s, mem, o_lag=O_LAG, side=iter(()), before_out=lambda: None):
        rows = pl.ds(pl.multiple_of(s * seg, seg), seg)
        xs = x_v[rows, :].astype(F32)
        h = jnp.concatenate([xs, mem], axis=0)

        def proj(j, p):
            y = _dot_tiles(h, w_all, (3 * p + j) * ntp, ntp)
            return jnp.concatenate([y[seg:], y[:seg]], axis=0)

        q, kb, vb, prob, att = {}, {}, {}, {}, {}
        acc = None
        for t in range(n_pair + V_LAG + 1):
            next(side, None)
            if t < n_pair:
                q[t] = proj(0, t)
                kb[t] = split_heads(proj(1, t))
            p = t - V_LAG
            if 0 <= p < n_pair:
                vb[p] = split_heads(proj(2, p))
            p = t - 1
            if 0 <= p < n_pair:
                prob[p] = softmax(_dot_nt(q.pop(p), kb.pop(p)))
            p = t - V_LAG - 1 - o_lag
            if p == 0 and o_lag != O_LAG:
                cp_wo(0).wait()
            if p >= 0:
                y = _dot(att.pop(p), wo_v[p * PW:(p + 1) * PW, :])
                acc = y if acc is None else acc + y
            p = t - V_LAG - 1
            if p >= 0:
                att[p] = _dot(prob.pop(p), vb.pop(p))
        before_out()
        rest = jnp.concatenate([att[p] for p in sorted(att)], axis=1)
        o = jnp.concatenate(
            [_dot(rest, wo_v[(n_pair - o_lag) * PW:, _tile(c)]) for c in range(nc)], axis=1)
        o = o if acc is None else acc + o
        out_v[rows, :] = (_gate(xs, gw) * o[M:] + gb_s[rows, :]).astype(out_v.dtype)
        return o[:M].astype(BF16).astype(F32)

    def store_out(s, n):
        rows = pl.ds(pl.multiple_of(s * seg, seg), n * seg)
        pltpu.make_async_copy(out_v.at[rows], out_hbm.at[rows], sem_out).start()

    def a_group(g, mem):
        s0 = 1 + g * A_UNROLL
        for u in range(A_UNROLL):
            mem = a_step(s0 + u, mem)
        store_out(s0, A_UNROLL)
        return mem

    def wait_wo():
        cp_wo(1).wait()

    mem = a_step(0, mem0_ref[...].astype(F32), n_pair // 2, b_tail(), wait_wo)
    store_out(0, 1)
    assert (n_seg - 1) % A_UNROLL == 0
    jax.lax.fori_loop(0, (n_seg - 1) // A_UNROLL, a_group, mem)
    pltpu.make_async_copy(out_v, out_hbm, sem_out).wait()


@functools.partial(jax.jit, static_argnames=("A_seg_len",))
def pallas_gated_mix__memory_aug_recurrent_mem_tr__sliding_local_dilated__prompt_kernel(
    A_x, A_mem0, A_Wq, A_Wk, A_Wv, A_Wo, A_seg_len, B_x, B_wqkv, B_wo, gate_w,
):
    del B_x
    B, S, D = A_x.shape
    M = A_mem0.shape[1]
    H, dh = A_Wq.shape[1:]
    seg = int(A_seg_len)
    L = M + seg
    assert B == 1 and S % (2 * B_ROWS) == 0 and S % seg == 0 and 2 * dh == 3 * LANES and 2 * L <= LANES
    nc = D // LANES

    def wt(w):
        return w.transpose(1, 2, 0).reshape(H * dh, D)

    hbm = pl.BlockSpec(memory_space=pl.ANY)
    vmem = pl.BlockSpec(memory_space=pltpu.VMEM)
    out = pl.pallas_call(
        functools.partial(_kernel, seg=seg, dh=dh),
        out_shape=jax.ShapeDtypeStruct((S, D), A_x.dtype),
        in_specs=[hbm, vmem, hbm, hbm, hbm, hbm, hbm, hbm, vmem],
        out_specs=hbm,
        scratch_shapes=[
            pltpu.VMEM((S, D), BF16),
            pltpu.VMEM((D, 3 * D), BF16),
            pltpu.VMEM((D, D), BF16),
            pltpu.VMEM((3 * D + B_HEADS, LANES), F32),
            pltpu.VMEM((nc, 3 * D // 2, LANES), jnp.uint32),
            pltpu.VMEM((nc, D // 2, LANES), jnp.uint32),
            pltpu.VMEM((3, (H + 4) * dh, D), BF16),
            pltpu.VMEM((3 * H * dh // LANES, D // 2, LANES), jnp.uint32),
            pltpu.VMEM((H * dh, D), BF16),
            *[pltpu.VMEM((B_ROWS, D), F32),
              pltpu.VMEM((nc, B_HALO + B_ROWS, LANES), F32),
              pltpu.VMEM((nc, B_HALO + B_ROWS, LANES), F32),
              pltpu.VMEM((B_ROWS, D), BF16)] * 2,
            pltpu.VMEM((S, D), F32),
            pltpu.VMEM((S, D), A_x.dtype),
            pltpu.SemaphoreType.DMA((2,)),
            pltpu.SemaphoreType.DMA((nc + 1,)),
            pltpu.SemaphoreType.DMA((4, S // (2 * B_ROWS))),
            pltpu.SemaphoreType.DMA(()),
        ],
        compiler_params=pltpu.CompilerParams(vmem_limit_bytes=112 * 2**20),
    )(A_x.reshape(S, D), A_mem0.reshape(M, D), wt(A_Wq), wt(A_Wk), wt(A_Wv),
      A_Wo.reshape(H * dh, D), B_wqkv, B_wo, gate_w)
    return out.reshape(B, S, D)
```
